```python
import jax
import jax.numpy as jnp

def _softmax(x, axis=-1):
    return jax.nn.softmax(x, axis=axis)
def _gelu(x):
    return jax.nn.gelu(x, approximate=True)
def _silu(x):
    return jax.nn.silu(x)
def _sigmoid(x):
    return jax.nn.sigmoid(x)
def _layernorm(x, axis=-1, eps=1e-5):
    m = jnp.mean(x, axis=axis, keepdims=True)
    v = jnp.var(x, axis=axis, keepdims=True)
    return (x - m) / jnp.sqrt(v + eps)
def _scatter_add(tgt, idx, src, axis=0):
    return tgt.at[idx].add(src)
def _segment_sum(src, seg, n):
    return jax.ops.segment_sum(src, seg, n)
class _Rng:
    def __init__(self, key):
        self._k = key
    def _next(self):
        self._k, sub = jax.random.split(self._k)
        return sub
    def normal(self, shape):
        return jax.random.normal(self._next(), shape, dtype=jnp.bfloat16)
    def randint(self, lo, hi, shape):
        return jax.random.randint(self._next(), shape, lo, hi, dtype=jnp.int32)
    def uniform(self, shape, lo=0.0, hi=1.0):
        return jax.random.uniform(self._next(), shape, jnp.bfloat16, lo, hi)
    def permutation(self, n):
        return jax.random.permutation(self._next(), n)


kernel_name = 'interleave_layers__sliding_block_cached__mixer_s_mlp__decode'

def setup_inputs():
    _rng = _Rng(jax.random.key(int.from_bytes(__import__("os").urandom(4), "little")))
    _w = (lambda a: (lambda t: t.astype(jnp.bfloat16) if jnp.issubdtype(t.dtype, jnp.floating) else t)(jnp.asarray(a)))
    def _A_setup():
        B, Sq, D = 1, 1, 640
        Hq, Hkv, Sk, Dh = 32, 32, 32768, 192
        assert Hq % Hkv == 0, (Hq, Hkv)
        return {
            "x": _w((lambda *s: _rng.normal(s) * 0.05)(B, Sq, D)),
            "k_cache": _w((lambda *s: _rng.normal(s) * 0.05)(B, Hkv, Sk, Dh)),
            "v_cache": _w((lambda *s: _rng.normal(s) * 0.05)(B, Hkv, Sk, Dh)),
            "wq": _w((lambda *s: _rng.normal(s) * 0.05)(D, Hq * Dh) * (D ** -0.5)),
            "wo": _w((lambda *s: _rng.normal(s) * 0.05)(Hq * Dh, D) * ((Hq * Dh) ** -0.5)),
        }
    _A_in = _A_setup()

    def _B_setup():
        B, S, D, F = 1, 1, 640, 1536
        return {
            "x":  _w((lambda *s: _rng.normal(s) * 0.05)(B, S, D)),
            "w1": _w((lambda *s: _rng.normal(s) * 0.05)(D, D) * (D ** -0.5)),
            "w2": _w((lambda *s: _rng.normal(s) * 0.05)(D, D) * (D ** -0.5)),
            "w3": _w((lambda *s: _rng.normal(s) * 0.05)(D, F) * (D ** -0.5)),
            "w4": _w((lambda *s: _rng.normal(s) * 0.05)(F, D) * (F ** -0.5)),
        }
    _B_in = _B_setup()

    return {
        "A_x": _A_in["x"],
        "A_k_cache": _A_in["k_cache"],
        "A_v_cache": _A_in["v_cache"],
        "A_wq": _A_in["wq"],
        "A_wo": _A_in["wo"],
        "B_x": _B_in["x"],
        "B_w1": _B_in["w1"],
        "B_w2": _B_in["w2"],
        "B_w3": _B_in["w3"],
        "B_w4": _B_in["w4"],
    }

def reference(A_x, A_k_cache, A_v_cache, A_wq, A_wo, B_x, B_w1, B_w2, B_w3, B_w4):
    def _A_ref(x, k_cache, v_cache, wq, wo):
        B, Sq, D = x.shape
        Hq, Dh = 32, 192
        Hkv, Sk = k_cache.shape[1], k_cache.shape[2]
        W = min(4096, max(256, Sk // 4))
        rep = Hq // Hkv
        q = (lambda x, *d: x.transpose(*d))((x @ wq).reshape(B, Sq, Hq, Dh), 0, 2, 1, 3)
        k = jnp.repeat(k_cache[:, :, Sk - W:, :], rep, axis=1)
        v = jnp.repeat(v_cache[:, :, Sk - W:, :], rep, axis=1)
        scores = jnp.einsum("bhqd,bhkd->bhqk", q, k) * (Dh ** -0.5)
        p = _softmax(scores, axis=-1)
        o = jnp.einsum("bhqk,bhkd->bhqd", p, v)
        return (lambda x, *d: x.transpose(*d))(o, 0, 2, 1, 3).reshape(B, Sq, Hq * Dh) @ wo

    def _B_ref(x, w1, w2, w3, w4):
        B, S, D = x.shape
        h = _gelu(_layernorm(x, axis=-1) @ w1)
        c = D // 4
        g0 = jnp.pad(h[:, :, 0*c:1*c], ((0, 0), (1, 0), (0, 0)))[:, :S, :]
        g1 = jnp.pad(h[:, :, 1*c:2*c], ((0, 0), (0, 1), (0, 0)))[:, 1:, :]
        g2 = jnp.pad(h[:, :, 2*c:3*c], ((0, 0), (2, 0), (0, 0)))[:, :S, :]
        g3 = jnp.pad(h[:, :, 3*c:   ], ((0, 0), (0, 2), (0, 0)))[:, 2:, :]
        hs = jnp.concatenate([g0, g1, g2, g3], axis=-1) @ w2
        x1 = x + hs
        h2 = _gelu(_layernorm(x1, axis=-1) @ w3) @ w4
        return x1 + h2

    x = A_x
    x = x + _A_ref(_layernorm(x, axis=-1), A_k_cache, A_v_cache, A_wq, A_wo)
    x = x + _B_ref(_layernorm(x, axis=-1), B_w1, B_w2, B_w3, B_w4)
    x = x + _A_ref(_layernorm(x, axis=-1), A_k_cache, A_v_cache, A_wq, A_wo)
    x = x + _B_ref(_layernorm(x, axis=-1), B_w1, B_w2, B_w3, B_w4)
    return x
```

```python
import jax
import jax.numpy as jnp
from jax import lax
import jax.experimental.pallas as pl
import jax.experimental.pallas.tpu as pltpu

D = 640
NH = 32
DH = 192
SK = 32768
W = 4096
F = 1536
L = 128
NP = NH // 2
NT = W // L
S0 = SK - W
EPS = 1e-5
SCALE = DH ** -0.5
NN = (((1,), (0,)), ((), ()))


def _ln(x):
    m = jnp.sum(x, axis=-1, keepdims=True) * (1.0 / D)
    d = x - m
    v = jnp.sum(d * d, axis=-1, keepdims=True) * (1.0 / D)
    return d * lax.rsqrt(v + EPS)


def _round_bf16(x):
    return x.astype(jnp.bfloat16).astype(jnp.float32)


def _mm(lhs, w32):
    return lax.dot_general(lhs, pltpu.bitcast(w32, jnp.bfloat16), NN,
                           preferred_element_type=jnp.float32)


def _kernel(x_hbm, k_hbm, v_hbm, wq_hbm, wo_hbm, w3_hbm, w4_hbm, o_ref,
            kb, vb, wq, wo, w3, w4, xb, qs, os_,
            sa0, sa1, sb0, sb1, p0, p1, acc0, acc1,
            ksem, vsem, wsem):
    kb16, vb16 = kb.bitcast(jnp.bfloat16), vb.bitcast(jnp.bfloat16)
    wq16, wo16 = wq.bitcast(jnp.bfloat16), wo.bitcast(jnp.bfloat16)
    w316, w416 = w3.bitcast(jnp.bfloat16), w4.bitcast(jnp.bfloat16)
    sa, sb, pb, acc = (sa0, sa1), (sb0, sb1), (p0, p1), (acc0, acc1)

    def start_cache(hbm, dst16, sem, ip):
        r0 = ip * (2 * DH)
        if not isinstance(ip, int):
            r0 = pl.multiple_of(r0, L)
        for j in range(NT):
            pltpu.make_async_copy(hbm.at[pl.ds(r0, 2 * DH), pl.ds(S0 + j * L, L)],
                                  dst16.at[ip, j], sem.at[ip]).start()

    def wait_cache(dst16, sem, ip):
        pltpu.make_async_copy(dst16.at[ip], dst16.at[ip], sem.at[ip]).wait()

    def start_weight(hbm, dst16, s):
        for n in range(dst16.shape[0]):
            pltpu.make_async_copy(hbm.at[:, pl.ds(n * L, L)], dst16.at[n], wsem.at[s]).start()

    def wait_weight(dst16, s):
        pltpu.make_async_copy(dst16, dst16, wsem.at[s]).wait()

    x_copy = pltpu.make_async_copy(x_hbm, xb, wsem.at[4])
    x_copy.start()
    start_weight(wq_hbm, wq16, 0)
    start_cache(k_hbm, kb16, ksem, 0)
    start_cache(k_hbm, kb16, ksem, 1)
    start_cache(v_hbm, vb16, vsem, 0)
    start_cache(k_hbm, kb16, ksem, 2)
    start_cache(v_hbm, vb16, vsem, 1)
    start_cache(k_hbm, kb16, ksem, 3)

    row = lax.broadcasted_iota(jnp.int32, (8, L), 0)
    lane = lax.broadcasted_iota(jnp.int32, (8, L), 1)
    mid_mask = (row % 2 == 0) == (lane < L // 2)

    def qk(ip, slot):
        lhs = [qs[ip * 3 + kt] for kt in range(3)]
        for j in range(NT):
            J, v = divmod(j, 4)
            r = [_mm(lhs[kt], kb[ip, j, kt * 64:(kt + 1) * 64, :]) for kt in range(3)]
            sa[slot][J, 2 * v:2 * v + 1, :] = r[0][2 * v:2 * v + 1, :]
            sb[slot][J, 2 * v:2 * v + 2, :] = r[1][2 * v:2 * v + 2, :]
            sa[slot][J, 2 * v + 1:2 * v + 2, :] = r[2][2 * v + 1:2 * v + 2, :]

    def per_head(t, op):
        t = op(t, pltpu.roll(t, 2, 0))
        return op(t, pltpu.roll(t, 4, 0))

    def softmax(slot):
        s = [(sa[slot][J] + sb[slot][J]) * SCALE for J in range(8)]
        m = s[0]
        for t in s[1:]:
            m = jnp.maximum(m, t)
        m = jnp.broadcast_to(jnp.max(m, axis=1, keepdims=True), (8, L))
        m = per_head(m, jnp.maximum)
        e = [jnp.exp(t - m) for t in s]
        tot = e[0]
        for t in e[1:]:
            tot = tot + t
        tot = jnp.broadcast_to(jnp.sum(tot, axis=1, keepdims=True), (8, L))
        inv = 1.0 / per_head(tot, jnp.add)
        for J in range(8):
            pb[slot][J] = e[J] * inv

    def pv(ip, slot):
        for h in range(2):
            a = None
            for j in range(NT):
                r = 2 * (j % 4) + h
                p = jnp.broadcast_to(pb[slot][j // 4, r:r + 1, :], (16, L))
                new = []
                for t in range(DH // 16):
                    w = vb[ip, j, h * 96 + t * 8:h * 96 + t * 8 + 8, :]
                    f = pltpu.bitcast(w, jnp.bfloat16).astype(jnp.float32) * p
                    new.append(f if a is None else a[t] + f)
                a = new
            for t in range(DH // 16):
                acc[slot][h * DH + t * 16:h * DH + t * 16 + 16, :] = a[t]

    def finalize(ip, slot):
        o = jnp.sum(acc[slot][...].T, axis=0, keepdims=True)
        o = jnp.broadcast_to(_round_bf16(o), (8, 2 * DH))
        for kt in range(3):
            os_[ip * 3 + kt] = o[:, kt * L:(kt + 1) * L]

    def layer(li, x):
        first = li == 0
        z = _round_bf16(_ln(x))

        @pl.when(first)
        def _():
            wait_weight(wq16, 0)
            wait_cache(kb16, ksem, 0)
            wait_cache(kb16, ksem, 1)

        for n in range(NH * DH // L):
            q = _round_bf16(_mm(z, wq[n]))
            qs[n] = jnp.where(mid_mask, q, 0.0) if n % 3 == 1 else q
        qk(0, 0)
        qk(1, 1)
        softmax(0)

        def stage(i, slot):
            @pl.when(first)
            def _():
                wait_cache(vb16, vsem, i)

                @pl.when(i + 2 < NP)
                def _():
                    wait_cache(kb16, ksem, i + 2)

                @pl.when(i + 2 < NP)
                def _():
                    start_cache(v_hbm, vb16, vsem, i + 2)

                @pl.when(i + 4 < NP)
                def _():
                    start_cache(k_hbm, kb16, ksem, i + 4)

                @pl.when(i == NP - 4)
                def _():
                    start_weight(wo_hbm, wo16, 1)

                @pl.when(i == NP - 3)
                def _():
                    start_weight(w3_hbm, w316, 2)
                    start_weight(w4_hbm, w416, 3)

            softmax(1 - slot)
            qk(jnp.minimum(i + 2, NP - 1), slot)
            pv(i, slot)
            finalize(jnp.maximum(i - 1, 0), 1 - slot)

        acc[1][...] = jnp.zeros(acc[1].shape, jnp.float32)

        def two_stages(t, c):
            stage(2 * t, 0)
            stage(2 * t + 1, 1)
            return c

        lax.fori_loop(0, NP // 2, two_stages, 0)
        finalize(NP - 1, 1)

        @pl.when(first)
        def _():
            wait_weight(wo16, 1)

        cols = []
        for n in range(D // L):
            parts = []
            for c in range(4):
                lhs = jnp.concatenate([os_[c * 12 + t] for t in range(12)], axis=1)
                parts.append(_mm(lhs, wo[n, c * 768:(c + 1) * 768, :]))
            cols.append((parts[0] + parts[1]) + (parts[2] + parts[3]))
        x = x + jnp.concatenate(cols, axis=1)

        y = _ln(x)
        y2 = _round_bf16(_ln(y))

        @pl.when(first)
        def _():
            wait_weight(w316, 2)

        h = jnp.concatenate([_mm(y2, w3[n]) for n in range(F // L)], axis=1)
        h = _round_bf16(jax.nn.gelu(h, approximate=True))

        @pl.when(first)
        def _():
            wait_weight(w416, 3)

        out = jnp.concatenate([_mm(h, w4[n]) for n in range(D // L)], axis=1)
        return x + (y + out)

    x_copy.wait()
    x0 = jnp.broadcast_to(xb[...].astype(jnp.float32), (8, D))
    x = lax.fori_loop(0, 2, layer, x0)
    o_ref[...] = x[:1].astype(o_ref.dtype)


@jax.jit
def pallas_interleave_layers__sliding_block_cached__mixer_s_mlp__decode_kernel(
    A_x: jax.Array,
    A_k_cache: jax.Array,
    A_v_cache: jax.Array,
    A_wq: jax.Array,
    A_wo: jax.Array,
    B_x: jax.Array,
    B_w1: jax.Array,
    B_w2: jax.Array,
    B_w3: jax.Array,
    B_w4: jax.Array,
):
    del B_x, B_w1, B_w2
    assert A_x.shape == (1, 1, D) and A_k_cache.shape == (1, NH, SK, DH)
    kt = jnp.swapaxes(A_k_cache, 2, 3).reshape(NH * DH, SK)
    vt = jnp.swapaxes(A_v_cache, 2, 3).reshape(NH * DH, SK)
    hbm = pl.BlockSpec(memory_space=pl.ANY)
    u32, f32 = jnp.uint32, jnp.float32
    out = pl.pallas_call(
        _kernel,
        out_shape=jax.ShapeDtypeStruct((1, D), A_x.dtype),
        in_specs=[hbm] * 7,
        scratch_shapes=[
            pltpu.VMEM((NP, NT, DH, L), u32),
            pltpu.VMEM((NP, NT, DH, L), u32),
            pltpu.VMEM((NH * DH // L, D // 2, L), u32),
            pltpu.VMEM((D // L, NH * DH // 2, L), u32),
            pltpu.VMEM((F // L, D // 2, L), u32),
            pltpu.VMEM((D // L, F // 2, L), u32),
            pltpu.VMEM((1, D), A_x.dtype),
            pltpu.VMEM((NH * DH // L, 8, L), f32),
            pltpu.VMEM((NH * DH // L, 8, L), f32),
            *[pltpu.VMEM((8, 8, L), f32)] * 6,
            *[pltpu.VMEM((2 * DH, L), f32)] * 2,
            pltpu.SemaphoreType.DMA((NP,)),
            pltpu.SemaphoreType.DMA((NP,)),
            pltpu.SemaphoreType.DMA((5,)),
        ],
        compiler_params=pltpu.CompilerParams(vmem_limit_bytes=120 * 2**20),
        name="interleave_decode",
    )(A_x.reshape(1, D), kt, vt, A_wq, A_wo, B_w3, B_w4)
    return out.reshape(1, 1, D)
```

```python
import jax
import jax.numpy as jnp
from jax import lax
import jax.experimental.pallas as pl
import jax.experimental.pallas.tpu as pltpu

D = 640
NH = 32
DH = 192
SK = 32768
W = 4096
F = 1536
L = 128
NP = NH // 2
NT = W // L
S0 = SK - W
EPS = 1e-5
SCALE = DH ** -0.5
NN = (((1,), (0,)), ((), ()))
GP = 2


def _ln(x):
    m = jnp.sum(x, axis=-1, keepdims=True) * (1.0 / D)
    d = x - m
    v = jnp.sum(d * d, axis=-1, keepdims=True) * (1.0 / D)
    return d * lax.rsqrt(v + EPS)


def _ln_twice(x):
    d = x - jnp.sum(x, axis=-1, keepdims=True) * (1.0 / D)
    m2 = jnp.sum(d, axis=-1, keepdims=True) * (1.0 / D)
    v = jnp.sum(d * d, axis=-1, keepdims=True) * (1.0 / D)
    r = lax.rsqrt(v + EPS)
    y = d * r
    v2 = (v - m2 * m2) * (r * r)
    return y, (y - m2 * r) * lax.rsqrt(v2 + EPS)


def _round_bf16(x):
    return x.astype(jnp.bfloat16).astype(jnp.float32)


def _mm(lhs, w32):
    return lax.dot_general(lhs, pltpu.bitcast(w32, jnp.bfloat16), NN,
                           preferred_element_type=jnp.float32)


def _kernel(x_hbm, k_hbm, v_hbm, wq_hbm, wo_hbm, w3_hbm, w4_hbm, o_ref,
            kb, vb, wq, wo, w3, w4, xb, qs, *rest):
    sa, sb, pb, acc = (rest[t * GP:(t + 1) * GP] for t in range(4))
    ksem, vsem, osem, wsem = rest[4 * GP:]
    kb16, vb16 = kb.bitcast(jnp.bfloat16), vb.bitcast(jnp.bfloat16)
    wq16, wo16 = wq.bitcast(jnp.bfloat16), wo.bitcast(jnp.bfloat16)
    w316, w416 = w3.bitcast(jnp.bfloat16), w4.bitcast(jnp.bfloat16)
    GR = GP * 2 * DH

    def start_cache(hbm, dst16, sem, ip):
        r0 = ip * (2 * DH)
        if not isinstance(ip, int):
            r0 = pl.multiple_of(r0, L)
        for j in range(NT):
            pltpu.make_async_copy(hbm.at[pl.ds(r0, 2 * DH), pl.ds(S0 + j * L, L)],
                                  dst16.at[ip, j], sem.at[ip]).start()

    def wait_cache(dst16, sem, ip):
        pltpu.make_async_copy(dst16.at[ip], dst16.at[ip], sem.at[ip]).wait()

    def start_weight(hbm, dst16, s, rows):
        for r in range(0, dst16.shape[1], rows):
            for n in range(dst16.shape[0]):
                pltpu.make_async_copy(hbm.at[pl.ds(r, rows), pl.ds(n * L, L)],
                                      dst16.at[n, pl.ds(r, rows)], wsem.at[s]).start()

    def wait_weight(dst16, s):
        pltpu.make_async_copy(dst16, dst16, wsem.at[s]).wait()

    def start_wo(g):
        for r in range(0, GR, 384):
            r0 = pl.multiple_of(g * GR + r, L)
            for n in range(D // L):
                pltpu.make_async_copy(wo_hbm.at[pl.ds(r0, 384), pl.ds(n * L, L)],
                                      wo16.at[g, n, pl.ds(r, 384)], osem.at[g]).start()

    def wait_wo(g):
        pltpu.make_async_copy(wo16.at[g], wo16.at[g], osem.at[g]).wait()

    x_copy = pltpu.make_async_copy(x_hbm, xb, wsem.at[3])
    x_copy.start()
    start_weight(wq_hbm, wq16, 0, D)
    for i in range(GP):
        start_cache(k_hbm, kb16, ksem, i)
    start_cache(v_hbm, vb16, vsem, 0)
    start_cache(k_hbm, kb16, ksem, GP)

    row = lax.broadcasted_iota(jnp.int32, (8, L), 0)
    lane = lax.broadcasted_iota(jnp.int32, (8, L), 1)
    mid_mask = (row % 2 == 0) == (lane < L // 2)

    def qproj(z, ip):
        for kt in range(3):
            q = _round_bf16(_mm(z, wq[ip * 3 + kt]))
            qs[ip * 3 + kt] = jnp.where(mid_mask, q, 0.0) if kt == 1 else q

    def qk(ip, slot):
        lhs = [qs[ip * 3 + kt] for kt in range(3)]
        for j in range(NT):
            J, v = divmod(j, 4)
            r = [_mm(lhs[kt], kb[ip, j, kt * 64:(kt + 1) * 64, :]) for kt in range(3)]
            sa[slot][J, 2 * v:2 * v + 1, :] = r[0][2 * v:2 * v + 1, :]
            sb[slot][J, 2 * v:2 * v + 2, :] = r[1][2 * v:2 * v + 2, :]
            sa[slot][J, 2 * v + 1:2 * v + 2, :] = r[2][2 * v + 1:2 * v + 2, :]

    def per_head(t, op):
        t = op(t, pltpu.roll(t, 2, 0))
        return op(t, pltpu.roll(t, 4, 0))

    def softmax(slot):
        s = [(sa[slot][J] + sb[slot][J]) * SCALE for J in range(8)]
        m = s[0]
        for t in s[1:]:
            m = jnp.maximum(m, t)
        m = jnp.broadcast_to(jnp.max(m, axis=1, keepdims=True), (8, L))
        m = per_head(m, jnp.maximum)
        e = [jnp.exp(t - m) for t in s]
        tot = e[0]
        for t in e[1:]:
            tot = tot + t
        tot = jnp.broadcast_to(jnp.sum(tot, axis=1, keepdims=True), (8, L))
        inv = 1.0 / per_head(tot, jnp.add)
        for J in range(8):
            pb[slot][J] = e[J] * inv

    def pv(ip, slot):
        for h in range(2):
            a = None
            for j in range(NT):
                r = 2 * (j % 4) + h
                p = jnp.broadcast_to(pb[slot][j // 4, r:r + 1, :], (16, L))
                new = []
                for t in range(DH // 16):
                    w = vb[ip, j, h * 96 + t * 8:h * 96 + t * 8 + 8, :]
                    f = pltpu.bitcast(w, jnp.bfloat16).astype(jnp.float32) * p
                    new.append(f if a is None else a[t] + f)
                a = new
            for t in range(DH // 16):
                acc[slot][h * DH + t * 16:h * DH + t * 16 + 16, :] = a[t]

    def finalize(slot):
        o = jnp.sum(acc[slot][...].T, axis=0, keepdims=True)
        return jnp.broadcast_to(_round_bf16(o), (8, 2 * DH))

    def layer(li, x):
        first = li == 0
        z = _round_bf16(_ln(x))

        @pl.when(first)
        def _():
            wait_weight(wq16, 0)
            for i in range(GP):
                wait_cache(kb16, ksem, i)
            start_cache(v_hbm, vb16, vsem, 1)

        for i in range(2 * GP):
            qproj(z, i)
        for i in range(GP):
            qk(i, i)
        for i in range(GP):
            softmax(i)

        def group(g, att):
            for slot in range(GP):
                i = g * GP + slot

                @pl.when(first)
                def _():
                    wait_cache(vb16, vsem, i)

                    @pl.when(i + GP + 1 < NP)
                    def _():
                        start_cache(k_hbm, kb16, ksem, i + GP + 1)

                    if slot == 0:
                        start_wo(g)

                    if slot == (NP - 2) % GP:
                        @pl.when(i == NP - 2)
                        def _():
                            start_weight(w3_hbm, w316, 1, 320)

                    if slot == (NP - 1) % GP:
                        @pl.when(i == NP - 1)
                        def _():
                            start_weight(w4_hbm, w416, 2, 256)

                    @pl.when(i + GP < NP)
                    def _():
                        wait_cache(kb16, ksem, i + GP)

                    @pl.when(i + 2 < NP)
                    def _():
                        start_cache(v_hbm, vb16, vsem, i + 2)

                pv(i, slot)
                qk(jnp.minimum(i + GP, NP - 1), slot)

            @pl.when(first)
            def _():
                wait_wo(g)

            o = jnp.concatenate([finalize(slot) for slot in range(GP)], axis=1)
            for slot in range(GP):
                qproj(z, jnp.minimum((g + 2) * GP + slot, NP - 1))
            for slot in range(GP):
                softmax(slot)
            return att + jnp.concatenate([_mm(o, wo[g, n]) for n in range(D // L)], axis=1)

        x = x + lax.fori_loop(0, NP // GP, group, jnp.zeros((8, D), jnp.float32))

        y, y2 = _ln_twice(x)
        y2 = _round_bf16(y2)

        @pl.when(first)
        def _():
            wait_weight(w316, 1)

        h = jnp.concatenate([_mm(y2, w3[n]) for n in range(F // L)], axis=1)
        h = _round_bf16(jax.nn.gelu(h, approximate=True))

        @pl.when(first)
        def _():
            wait_weight(w416, 2)

        out = jnp.concatenate([_mm(h, w4[n]) for n in range(D // L)], axis=1)
        return x + (y + out)

    x_copy.wait()
    x0 = jnp.broadcast_to(xb[...].astype(jnp.float32), (8, D))
    x = lax.fori_loop(0, 2, layer, x0)
    o_ref[...] = x[:1].astype(o_ref.dtype)


@jax.jit
def pallas_interleave_layers__sliding_block_cached__mixer_s_mlp__decode_kernel(
    A_x: jax.Array,
    A_k_cache: jax.Array,
    A_v_cache: jax.Array,
    A_wq: jax.Array,
    A_wo: jax.Array,
    B_x: jax.Array,
    B_w1: jax.Array,
    B_w2: jax.Array,
    B_w3: jax.Array,
    B_w4: jax.Array,
):
    del B_x, B_w1, B_w2
    assert A_x.shape == (1, 1, D) and A_k_cache.shape == (1, NH, SK, DH)
    kt = jnp.swapaxes(A_k_cache, 2, 3).reshape(NH * DH, SK)
    vt = jnp.swapaxes(A_v_cache, 2, 3).reshape(NH * DH, SK)
    hbm = pl.BlockSpec(memory_space=pl.ANY)
    u32, f32 = jnp.uint32, jnp.float32
    out = pl.pallas_call(
        _kernel,
        out_shape=jax.ShapeDtypeStruct((1, D), A_x.dtype),
        in_specs=[hbm] * 7,
        scratch_shapes=[
            pltpu.VMEM((NP, NT, DH, L), u32),
            pltpu.VMEM((NP, NT, DH, L), u32),
            pltpu.VMEM((NH * DH // L, D // 2, L), u32),
            pltpu.VMEM((NP // GP, D // L, GP * DH, L), u32),
            pltpu.VMEM((F // L, D // 2, L), u32),
            pltpu.VMEM((D // L, F // 2, L), u32),
            pltpu.VMEM((1, D), A_x.dtype),
            pltpu.VMEM((NH * DH // L, 8, L), f32),
            *[pltpu.VMEM((8, 8, L), f32)] * (3 * GP),
            *[pltpu.VMEM((2 * DH, L), f32)] * GP,
            pltpu.SemaphoreType.DMA((NP,)),
            pltpu.SemaphoreType.DMA((NP,)),
            pltpu.SemaphoreType.DMA((NP // GP,)),
            pltpu.SemaphoreType.DMA((4,)),
        ],
        compiler_params=pltpu.CompilerParams(
            vmem_limit_bytes=120 * 2**20,
            disable_bounds_checks=True,
            disable_semaphore_checks=True,
        ),
        name="interleave_decode",
    )(A_x.reshape(1, D), kt, vt, A_wq, A_wo, B_w3, B_w4)
    return out.reshape(1, 1, D)
```

```python
import jax
import jax.numpy as jnp
from jax import lax
import jax.experimental.pallas as pl
import jax.experimental.pallas.tpu as pltpu

D = 640
NH = 32
DH = 192
SK = 32768
W = 4096
F = 1536
L = 128
NP = NH // 2
NT = W // L
S0 = SK - W
EPS = 1e-5
SCALE = DH ** -0.5
NN = (((1,), (0,)), ((), ()))
U = 4


def _ln(x):
    m = jnp.sum(x, axis=-1, keepdims=True) * (1.0 / D)
    d = x - m
    v = jnp.sum(d * d, axis=-1, keepdims=True) * (1.0 / D)
    return d * lax.rsqrt(v + EPS)


def _ln_twice(x):
    d = x - jnp.sum(x, axis=-1, keepdims=True) * (1.0 / D)
    m2 = jnp.sum(d, axis=-1, keepdims=True) * (1.0 / D)
    v = jnp.sum(d * d, axis=-1, keepdims=True) * (1.0 / D)
    r = lax.rsqrt(v + EPS)
    y = d * r
    v2 = (v - m2 * m2) * (r * r)
    return y, (y - m2 * r) * lax.rsqrt(v2 + EPS)


def _round_bf16(x):
    return x.astype(jnp.bfloat16).astype(jnp.float32)


def _mm(lhs, w32):
    return lax.dot_general(lhs, pltpu.bitcast(w32, jnp.bfloat16), NN,
                           preferred_element_type=jnp.float32)


def _kernel(x_hbm, k_hbm, v_hbm, wq_hbm, wo_hbm, w3_hbm, w4_hbm, o_ref,
            kb, vb, wq, wo, w3, w4, xb, qs, opart, *rest):
    sa, sb, lb, rest = rest[0:4], rest[4:8], rest[8:12], rest[12:]
    mb, pb, acc, ob, qpart, rest = (*(rest[2 * t:2 * t + 2] for t in range(5)), rest[10:])
    ksem, vsem, osem, wsem = rest
    kb16, vb16 = kb.bitcast(jnp.bfloat16), vb.bitcast(jnp.bfloat16)
    wq16, wo16 = wq.bitcast(jnp.bfloat16), wo.bitcast(jnp.bfloat16)
    w316, w416 = w3.bitcast(jnp.bfloat16), w4.bitcast(jnp.bfloat16)
    PR = 2 * DH

    def pair_row(ip):
        return ip * PR if isinstance(ip, int) else pl.multiple_of(ip * PR, L)

    def start_cache(hbm, dst16, sem, ip):
        r0 = pair_row(ip)
        for j in range(NT):
            pltpu.make_async_copy(hbm.at[pl.ds(r0, PR), pl.ds(S0 + j * L, L)],
                                  dst16.at[ip, j], sem.at[ip]).start()

    def start_wo(ip):
        r0 = pair_row(ip)
        for n in range(D // L):
            pltpu.make_async_copy(wo_hbm.at[pl.ds(r0, PR), pl.ds(n * L, L)],
                                  wo16.at[ip, n], osem.at[ip]).start()

    def wait_slab(dst16, sem, ip):
        pltpu.make_async_copy(dst16.at[ip], dst16.at[ip], sem.at[ip]).wait()

    def start_weight(hbm, dst16, s, rows):
        for r in range(0, dst16.shape[1], rows):
            for n in range(dst16.shape[0]):
                pltpu.make_async_copy(hbm.at[pl.ds(r, rows), pl.ds(n * L, L)],
                                      dst16.at[n, pl.ds(r, rows)], wsem.at[s]).start()

    def wait_weight(dst16, s):
        pltpu.make_async_copy(dst16, dst16, wsem.at[s]).wait()

    x_copy = pltpu.make_async_copy(x_hbm, xb, wsem.at[3])
    x_copy.start()
    start_weight(wq_hbm, wq16, 0, D)
    for i in range(3):
        start_cache(k_hbm, kb16, ksem, i)
    start_cache(v_hbm, vb16, vsem, 0)
    start_cache(k_hbm, kb16, ksem, 3)

    row = lax.broadcasted_iota(jnp.int32, (8, L), 0)
    lane = lax.broadcasted_iota(jnp.int32, (8, L), 1)
    mid_mask = (row % 2 == 0) == (lane < L // 2)

    def put_q(ip, n, q):
        q = _round_bf16(q)
        qs[ip * 3 + n] = jnp.where(mid_mask, q, 0.0) if n == 1 else q

    def q_partials(z, ip, buf):
        for n in range(3):
            for kt in range(D // L):
                buf[n * 5 + kt] = _mm(z[:, kt * L:(kt + 1) * L],
                                      wq[ip * 3 + n, kt * 64:(kt + 1) * 64, :])

    def q_sum(ip, buf):
        for n in range(3):
            t = [buf[n * 5 + kt] for kt in range(D // L)]
            put_q(ip, n, (t[0] + t[1]) + (t[2] + t[3]) + t[4])

    def qk(ip, a_ref, b_ref):
        lhs = [qs[ip * 3 + kt] for kt in range(3)]
        for j in range(NT):
            J, v = divmod(j, 4)
            r = [_mm(lhs[kt], kb[ip, j, kt * 64:(kt + 1) * 64, :]) for kt in range(3)]
            a_ref[J, 2 * v:2 * v + 1, :] = r[0][2 * v:2 * v + 1, :]
            b_ref[J, 2 * v:2 * v + 2, :] = r[1][2 * v:2 * v + 2, :]
            a_ref[J, 2 * v + 1:2 * v + 2, :] = r[2][2 * v + 1:2 * v + 2, :]

    def per_head(t, op):
        t = op(t, pltpu.roll(t, 2, 0))
        return op(t, pltpu.roll(t, 4, 0))

    def score_max(a_ref, b_ref, m_ref):
        s = [(a_ref[J] + b_ref[J]) * SCALE for J in range(8)]
        m = s[0]
        for t in s[1:]:
            m = jnp.maximum(m, t)
        for J in range(8):
            a_ref[J] = s[J]
        m_ref[...] = jnp.broadcast_to(jnp.max(m, axis=1, keepdims=True), (8, L))

    def score_exp(a_ref, m_ref, p_ref, l_ref):
        m = per_head(m_ref[...], jnp.maximum)
        e = [jnp.exp(a_ref[J] - m) for J in range(8)]
        tot = e[0]
        for t in e[1:]:
            tot = tot + t
        for J in range(8):
            p_ref[J] = e[J]
        l_ref[...] = jnp.broadcast_to(jnp.sum(tot, axis=1, keepdims=True), (8, L))

    def pv(ip, p_ref, acc_ref):
        for h in range(2):
            a = None
            for j in range(NT):
                r = 2 * (j % 4) + h
                p = jnp.broadcast_to(p_ref[j // 4, r:r + 1, :], (16, L))
                new = []
                for t in range(DH // 16):
                    w = vb[ip, j, h * 96 + t * 8:h * 96 + t * 8 + 8, :]
                    f = pltpu.bitcast(w, jnp.bfloat16).astype(jnp.float32) * p
                    new.append(f if a is None else a[t] + f)
                a = new
            for t in range(DH // 16):
                acc_ref[h * DH + t * 16:h * DH + t * 16 + 16, :] = a[t]

    def finalize(acc_ref, l_ref):
        o = jnp.sum(acc_ref[...].T, axis=0, keepdims=True)
        o = jnp.broadcast_to(o, (8, PR))
        inv = 1.0 / per_head(l_ref[...], jnp.add)
        i0, i1 = jnp.broadcast_to(inv[0:1], (8, L)), jnp.broadcast_to(inv[1:2], (8, L))
        sc = (i0, jnp.where(lane < L // 2, i0, i1), i1)
        return [_round_bf16(o[:, kt * L:(kt + 1) * L] * sc[kt]) for kt in range(3)]

    def o_partials(ip, o_tiles):
        for kt in range(3):
            lhs = o_tiles[kt]
            for n in range(D // L):
                opart[ip * 15 + kt * 5 + n] = _mm(lhs, wo[ip, n, kt * 64:(kt + 1) * 64, :])

    def layer(li, x):
        first = li == 0
        z = _round_bf16(_ln(x))

        @pl.when(first)
        def _():
            wait_weight(wq16, 0)
            for i in range(3):
                wait_slab(kb16, ksem, i)
            start_cache(v_hbm, vb16, vsem, 1)

        for i in range(4):
            for n in range(3):
                put_q(i, n, _mm(z, wq[i * 3 + n]))
        q_partials(z, 4, qpart[0])
        for i in range(3):
            qk(i, sa[i], sb[i])
        score_max(sa[0], sb[0], mb[0])
        score_max(sa[1], sb[1], mb[1])
        score_exp(sa[0], mb[0], pb[0], lb[0])
        acc[1][...] = jnp.zeros(acc[1].shape, jnp.float32)
        lb[3][...] = jnp.ones(lb[3].shape, jnp.float32)
        ob[0][...] = jnp.zeros(ob[0].shape, jnp.float32)

        def stages(t, c):
            for u in range(U):
                i = t * U + u

                @pl.when(first)
                def _():
                    wait_slab(vb16, vsem, i)

                    @pl.when(i + 4 < NP)
                    def _():
                        start_cache(k_hbm, kb16, ksem, i + 4)

                    start_wo(i)

                    @pl.when(i >= 2)
                    def _():
                        wait_slab(wo16, osem, i - 2)

                    if u == (NP - 2) % U:
                        @pl.when(i == NP - 2)
                        def _():
                            start_weight(w3_hbm, w316, 1, 320)

                    if u == (NP - 1) % U:
                        @pl.when(i == NP - 1)
                        def _():
                            start_weight(w4_hbm, w416, 2, 256)

                    @pl.when(i + 3 < NP)
                    def _():
                        wait_slab(kb16, ksem, i + 3)

                    @pl.when(i + 2 < NP)
                    def _():
                        start_cache(v_hbm, vb16, vsem, i + 2)

                o = finalize(acc[(u + 1) % 2], lb[(u + 3) % 4])
                for kt in range(3):
                    ob[(u + 1) % 2][kt] = o[kt]
                pv(i, pb[u % 2], acc[u % 2])
                qk(jnp.minimum(i + 3, NP - 1), sa[(u + 3) % 4], sb[(u + 3) % 4])
                o_partials(jnp.maximum(i - 2, 0), [ob[u % 2][kt] for kt in range(3)])
                score_max(sa[(u + 2) % 4], sb[(u + 2) % 4], mb[u % 2])
                score_exp(sa[(u + 1) % 4], mb[(u + 1) % 2], pb[(u + 1) % 2], lb[(u + 1) % 4])
                q_partials(z, jnp.minimum(i + 5, NP - 1), qpart[(u + 1) % 2])
                q_sum(jnp.minimum(i + 4, NP - 1), qpart[u % 2])
            return c

        lax.fori_loop(0, NP // U, stages, 0)

        @pl.when(first)
        def _():
            wait_slab(wo16, osem, NP - 2)
            wait_slab(wo16, osem, NP - 1)

        o15 = finalize(acc[1], lb[3])
        o14 = [ob[0][kt] for kt in range(3)]
        cols = []
        for n in range(D // L):
            parts = [opart[t * 5 + n] for t in range(3 * (NP - 2))]
            while len(parts) > 1:
                parts = [sum(parts[k:k + 2][1:], parts[k]) for k in range(0, len(parts), 2)]
            last = [_mm(jnp.concatenate(o, axis=1), wo[ip, n]) for ip, o in ((NP - 2, o14), (NP - 1, o15))]
            cols.append((parts[0] + last[0]) + last[1])
        x = x + jnp.concatenate(cols, axis=1)

        y, y2 = _ln_twice(x)
        y2 = _round_bf16(y2)

        @pl.when(first)
        def _():
            wait_weight(w316, 1)

        h = jnp.concatenate([_mm(y2, w3[n]) for n in range(F // L)], axis=1)
        h = _round_bf16(jax.nn.gelu(h, approximate=True))

        @pl.when(first)
        def _():
            wait_weight(w416, 2)

        out = jnp.concatenate([_mm(h, w4[n]) for n in range(D // L)], axis=1)
        return x + (y + out)

    x_copy.wait()
    x0 = jnp.broadcast_to(xb[...].astype(jnp.float32), (8, D))
    x = lax.fori_loop(0, 2, layer, x0)
    o_ref[...] = x[:1].astype(o_ref.dtype)


@jax.jit
def pallas_interleave_layers__sliding_block_cached__mixer_s_mlp__decode_kernel(
    A_x: jax.Array,
    A_k_cache: jax.Array,
    A_v_cache: jax.Array,
    A_wq: jax.Array,
    A_wo: jax.Array,
    B_x: jax.Array,
    B_w1: jax.Array,
    B_w2: jax.Array,
    B_w3: jax.Array,
    B_w4: jax.Array,
):
    del B_x, B_w1, B_w2
    assert A_x.shape == (1, 1, D) and A_k_cache.shape == (1, NH, SK, DH)
    kt = jnp.swapaxes(A_k_cache, 2, 3).reshape(NH * DH, SK)
    vt = jnp.swapaxes(A_v_cache, 2, 3).reshape(NH * DH, SK)
    hbm = pl.BlockSpec(memory_space=pl.ANY)
    u32, f32 = jnp.uint32, jnp.float32
    out = pl.pallas_call(
        _kernel,
        out_shape=jax.ShapeDtypeStruct((1, D), A_x.dtype),
        in_specs=[hbm] * 7,
        scratch_shapes=[
            pltpu.VMEM((NP, NT, DH, L), u32),
            pltpu.VMEM((NP, NT, DH, L), u32),
            pltpu.VMEM((NH * DH // L, D // 2, L), u32),
            pltpu.VMEM((NP, D // L, DH, L), u32),
            pltpu.VMEM((F // L, D // 2, L), u32),
            pltpu.VMEM((D // L, F // 2, L), u32),
            pltpu.VMEM((1, D), A_x.dtype),
            pltpu.VMEM((NH * DH // L, 8, L), f32),
            pltpu.VMEM((NP * 15, 8, L), f32),
            *[pltpu.VMEM((8, 8, L), f32)] * 8,
            *[pltpu.VMEM((8, L), f32)] * 6,
            *[pltpu.VMEM((8, 8, L), f32)] * 2,
            *[pltpu.VMEM((2 * DH, L), f32)] * 2,
            *[pltpu.VMEM((3, 8, L), f32)] * 2,
            *[pltpu.VMEM((15, 8, L), f32)] * 2,
            pltpu.SemaphoreType.DMA((NP,)),
            pltpu.SemaphoreType.DMA((NP,)),
            pltpu.SemaphoreType.DMA((NP,)),
            pltpu.SemaphoreType.DMA((4,)),
        ],
        compiler_params=pltpu.CompilerParams(
            vmem_limit_bytes=120 * 2**20,
            disable_bounds_checks=True,
            disable_semaphore_checks=True,
        ),
        name="interleave_decode",
    )(A_x.reshape(1, D), kt, vt, A_wq, A_wo, B_w3, B_w4)
    return out.reshape(1, 1, D)
```

```python
import jax
X = 'xfpaqo12bg'; XL = 'xfpon12g'
import jax.numpy as jnp
from jax import lax
import jax.experimental.pallas as pl
import jax.experimental.pallas.tpu as pltpu

D = 640
NH = 32
DH = 192
SK = 32768
W = 4096
F = 1536
L = 128
NP = NH // 2
NT = W // L
S0 = SK - W
EPS = 1e-5
SCALE = DH ** -0.5
NN = (((1,), (0,)), ((), ()))
NTD = (((1,), (1,)), ((), ()))
U = 4


def _ln(x):
    m = jnp.sum(x, axis=-1, keepdims=True) * (1.0 / D)
    d = x - m
    v = jnp.sum(d * d, axis=-1, keepdims=True) * (1.0 / D)
    return d * lax.rsqrt(v + EPS)


def _ln_twice(x):
    d = x - jnp.sum(x, axis=-1, keepdims=True) * (1.0 / D)
    m2 = jnp.sum(d, axis=-1, keepdims=True) * (1.0 / D)
    v = jnp.sum(d * d, axis=-1, keepdims=True) * (1.0 / D)
    r = lax.rsqrt(v + EPS)
    y = d * r
    v2 = (v - m2 * m2) * (r * r)
    return y, (y - m2 * r) * lax.rsqrt(v2 + EPS)


def _round_bf16(x):
    return x.astype(jnp.bfloat16).astype(jnp.float32)


def _mm(lhs, w32):
    return lax.dot_general(lhs, pltpu.bitcast(w32, jnp.bfloat16), NN,
                           preferred_element_type=jnp.float32)


def _when(cond):
    if isinstance(cond, bool):
        return (lambda f: f()) if cond else (lambda f: None)
    return pl.when(cond)


def _kernel(x_hbm, k_hbm, v_hbm, wq_hbm, wo_hbm, w3_hbm, w4_hbm, o_ref,
            kb, vb, wq, wo, w3, w4, xb, qs, opart, *rest):
    sa, sb, lb, mb, rest = rest[0:4], rest[4:8], rest[8:12], rest[12:16], rest[16:]
    pb, acc, ob, qpart, tb, rest = (*(rest[2 * t:2 * t + 2] for t in range(5)), rest[10:])
    nb, (ksem, vsem, osem, wsem) = rest[:U], rest[U:]
    kb16, vb16 = kb.bitcast(jnp.bfloat16), vb.bitcast(jnp.bfloat16)
    wq16, wo16 = wq.bitcast(jnp.bfloat16), wo.bitcast(jnp.bfloat16)
    w316, w416 = w3.bitcast(jnp.bfloat16), w4.bitcast(jnp.bfloat16)
    PR = 2 * DH

    def pair_row(ip):
        return ip * PR if isinstance(ip, int) else pl.multiple_of(ip * PR, L)

    def start_cache(hbm, dst16, sem, ip):
        r0 = pair_row(ip)
        for j in range(NT):
            pltpu.make_async_copy(hbm.at[pl.ds(r0, PR), pl.ds(S0 + j * L, L)],
                                  dst16.at[ip, j], sem.at[ip]).start()

    def start_wo(ip):
        r0 = pair_row(ip)
        for n in range(D // L):
            pltpu.make_async_copy(wo_hbm.at[pl.ds(r0, PR), pl.ds(n * L, L)],
                                  wo16.at[ip, n], osem.at[ip]).start()

    def wait_slab(dst16, sem, ip):
        pltpu.make_async_copy(dst16.at[ip], dst16.at[ip], sem.at[ip]).wait()

    def start_weight(hbm, dst16, s, rows):
        for r in range(0, dst16.shape[1], rows):
            for n in range(dst16.shape[0]):
                pltpu.make_async_copy(hbm.at[pl.ds(r, rows), pl.ds(n * L, L)],
                                      dst16.at[n, pl.ds(r, rows)], wsem.at[s]).start()

    def wait_weight(dst16, s):
        pltpu.make_async_copy(dst16, dst16, wsem.at[s]).wait()

    x_copy = pltpu.make_async_copy(x_hbm, xb, wsem.at[3])
    x_copy.start()
    start_weight(wq_hbm, wq16, 0, D)
    for i in range(4):
        start_cache(k_hbm, kb16, ksem, i)
    start_cache(v_hbm, vb16, vsem, 0)
    start_cache(k_hbm, kb16, ksem, 4)

    row = lax.broadcasted_iota(jnp.int32, (8, L), 0)
    lane = lax.broadcasted_iota(jnp.int32, (8, L), 1)
    mid_mask = (row % 2 == 0) == (lane < L // 2)

    def put_q(ip, n, q):
        q = _round_bf16(q)
        qs[ip * 3 + n] = jnp.where(mid_mask, q, 0.0) if n == 1 else q

    def q_partials(z, ip, buf):
        for n in range(3):
            for kt in range(D // L):
                buf[n * 5 + kt] = _mm(z[:, kt * L:(kt + 1) * L],
                                      wq[ip * 3 + n, kt * 64:(kt + 1) * 64, :])

    def q_sum(ip, buf):
        for n in range(3):
            t = [buf[n * 5 + kt] for kt in range(D // L)]
            put_q(ip, n, (t[0] + t[1]) + (t[2] + t[3]) + t[4])

    def qk(ip, a_ref, b_ref):
        lhs = [qs[ip * 3 + kt] for kt in range(3)]
        for j in range(NT):
            J, v = divmod(j, 4)
            r = [_mm(lhs[kt], kb[ip, j, kt * 64:(kt + 1) * 64, :]) for kt in range(3)]
            a_ref[J, 2 * v:2 * v + 1, :] = r[0][2 * v:2 * v + 1, :]
            b_ref[J, 2 * v:2 * v + 2, :] = r[1][2 * v:2 * v + 2, :]
            a_ref[J, 2 * v + 1:2 * v + 2, :] = r[2][2 * v + 1:2 * v + 2, :]

    def per_head(t, op):
        t = op(t, pltpu.roll(t, 2, 0))
        return op(t, pltpu.roll(t, 4, 0))

    def score_max(a_ref, b_ref, m_ref):
        s = [(a_ref[J] + b_ref[J]) * SCALE for J in range(8)]
        m = s[0]
        for t in s[1:]:
            m = jnp.maximum(m, t)
        for J in range(8):
            a_ref[J] = s[J]
        m_ref[...] = m

    def lane_max(m_ref):
        m_ref[...] = jnp.broadcast_to(jnp.max(m_ref[...], axis=1, keepdims=True), (8, L))

    def lane_sum(l_ref):
        l_ref[...] = jnp.broadcast_to(jnp.sum(l_ref[...], axis=1, keepdims=True), (8, L))

    def score_exp(a_ref, m_ref, p_ref, l_ref):
        m = per_head(m_ref[...], jnp.maximum)
        e = [jnp.exp(a_ref[J] - m) for J in range(8)]
        tot = e[0]
        for t in e[1:]:
            tot = tot + t
        for J in range(8):
            p_ref[J] = e[J]
        l_ref[...] = tot

    def pv(ip, p_ref, acc_ref, rows=PR):
        for h in range(2):
            nt = min(DH, rows - h * DH) // 16
            a = None
            for j in range(NT):
                r = 2 * (j % 4) + h
                p = jnp.broadcast_to(p_ref[j // 4, r:r + 1, :], (16, L))
                new = []
                for t in range(nt):
                    w = vb[ip, j, h * 96 + t * 8:h * 96 + t * 8 + 8, :]
                    f = pltpu.bitcast(w, jnp.bfloat16).astype(jnp.float32) * p
                    new.append(f if a is None else a[t] + f)
                a = new
            for t in range(nt):
                acc_ref[h * DH + t * 16:h * DH + t * 16 + 16, :] = a[t]

    def pv_mxu(ip, p_ref, n_ref):
        for J in range(8):
            lhs = _round_bf16(p_ref[J])
            for v in range(4):
                w = pltpu.bitcast(vb[ip, 4 * J + v, 128:192, :], jnp.bfloat16)
                r = lax.dot_general(lhs, w, NTD, preferred_element_type=jnp.float32)
                n_ref[J, 2 * v + 1:2 * v + 2, :] = r[2 * v + 1:2 * v + 2, :]

    def transpose_acc(acc_ref, t_ref, tiles=3):
        for kt in range(tiles):
            t_ref[kt] = acc_ref[kt * L:(kt + 1) * L, :].T

    def finalize(t_ref, l_ref, n_ref=None):
        o = [jnp.sum(t_ref[kt], axis=0, keepdims=True) for kt in range(3 if n_ref is None else 2)]
        if n_ref is not None:
            t = [jnp.where(row % 2 == 1, n_ref[J], 0.0) for J in range(8)]
            t = ((t[0] + t[1]) + (t[2] + t[3])) + ((t[4] + t[5]) + (t[6] + t[7]))
            o.append(jnp.sum(t, axis=0, keepdims=True))
        o = jnp.concatenate(o, axis=1)
        o = jnp.broadcast_to(o, (8, PR))
        inv = 1.0 / per_head(l_ref[...], jnp.add)
        i0, i1 = jnp.broadcast_to(inv[0:1], (8, L)), jnp.broadcast_to(inv[1:2], (8, L))
        sc = (i0, jnp.where(lane < L // 2, i0, i1), i1)
        return [_round_bf16(o[:, kt * L:(kt + 1) * L] * sc[kt]) for kt in range(3)]

    def o_partials(ip, o_tiles):
        for kt in range(3):
            lhs = o_tiles[kt]
            for n in range(D // L):
                opart[ip * 15 + kt * 5 + n] = _mm(lhs, wo[ip, n, kt * 64:(kt + 1) * 64, :])

    def layer(li, x):
        first = li == 0
        z = _round_bf16(_ln(x))

        @pl.when(first)
        def _():
            wait_weight(wq16, 0)
            for i in range(4):
                wait_slab(kb16, ksem, i)
            start_cache(v_hbm, vb16, vsem, 1)

        for i in range(5):
            for n in range(3):
                put_q(i, n, _mm(z, wq[i * 3 + n]))
        q_partials(z, 5, qpart[0])
        for i in range(4):
            qk(i, sa[i], sb[i])
        for i in range(3):
            score_max(sa[i], sb[i], mb[i])
        for i in range(2):
            lane_max(mb[i])
        score_exp(sa[0], mb[0], pb[0], lb[0])
        acc[1][...] = jnp.zeros(acc[1].shape, jnp.float32)
        tb[0][...] = jnp.zeros(tb[0].shape, jnp.float32)
        lb[2][...] = jnp.ones(lb[2].shape, jnp.float32)
        lb[3][...] = jnp.ones(lb[3].shape, jnp.float32)
        ob[1][...] = jnp.zeros(ob[1].shape, jnp.float32)

        def stage(i, u, last):
            if True:

                @pl.when(first)
                def _():
                    wait_slab(vb16, vsem, i)

                    @_when(i + 5 < NP)
                    def _():
                        start_cache(k_hbm, kb16, ksem, i + 5)

                    start_wo(i)

                    @_when(i >= 3)
                    def _():
                        wait_slab(wo16, osem, i - 3)

                    if last and u == (NP - 2) % U:
                        @_when(i == NP - 2)
                        def _():
                            start_weight(w3_hbm, w316, 1, 320)

                    if last and u == (NP - 1) % U:
                        @_when(i == NP - 1)
                        def _():
                            start_weight(w4_hbm, w416, 2, 256)

                    @_when(i + 4 < NP)
                    def _():
                        wait_slab(kb16, ksem, i + 4)

                    @_when(i + 2 < NP)
                    def _():
                        start_cache(v_hbm, vb16, vsem, i + 2)

                for c_ in (XL if last else X):
                    if c_ == "f":
                        transpose_acc(acc[(u + 1) % 2], tb[(u + 1) % 2], 2 if last and u >= 1 else 3)
                    if c_ == "g":
                        o = finalize(tb[u % 2], lb[(u + 2) % 4], nb[u - 2] if last and u >= 2 else None)
                        for kt in range(3):
                            ob[u % 2][kt] = o[kt]
                    if c_ == "p":
                        pv(i, pb[u % 2], acc[u % 2], 2 * L if last else PR)
                    if c_ == "n":
                        pv_mxu(i, pb[u % 2], nb[u])
                    if c_ == "q":
                        qk(jnp.minimum(i + 4, NP - 1), sa[u % 4], sb[u % 4])
                    if c_ == "1" and (not last or u < 1):
                        score_max(sa[(u + 3) % 4], sb[(u + 3) % 4], mb[(u + 3) % 4])
                    if c_ == "x":
                        if not last or u < 2:
                            lane_max(mb[(u + 2) % 4])
                        lane_sum(lb[u % 4])
                    if c_ == "2" and (not last or u < 3):
                        score_exp(sa[(u + 1) % 4], mb[(u + 1) % 4], pb[(u + 1) % 2], lb[(u + 1) % 4])
                    if c_ == "a":
                        q_partials(z, jnp.minimum(i + 6, NP - 1), qpart[(u + 1) % 2])
                    if c_ == "b":
                        q_sum(jnp.minimum(i + 5, NP - 1), qpart[u % 2])
                    if c_ == "o":
                        o_partials((i - 3 if last else jnp.maximum(i - 3, 0)), [ob[(u + 1) % 2][kt] for kt in range(3)])

        def stages(t, c):
            for u in range(U):
                stage(t * U + u, u, False)
            return c

        lax.fori_loop(0, NP // U - 1, stages, 0)
        for u in range(U):
            stage(NP - U + u, u, True)

        @pl.when(first)
        def _():
            for ip in range(NP - 3, NP):
                wait_slab(wo16, osem, ip)

        transpose_acc(acc[1], tb[1], 2)
        tail = ([ob[1][kt] for kt in range(3)],
                finalize(tb[0], lb[2], nb[2]), finalize(tb[1], lb[3], nb[3]))
        cols = []
        for n in range(D // L):
            parts = [opart[t * 5 + n] for t in range(3 * (NP - 3))]
            while len(parts) > 1:
                parts = [sum(parts[k:k + 2][1:], parts[k]) for k in range(0, len(parts), 2)]
            last = [_mm(jnp.concatenate(o, axis=1), wo[NP - 3 + k, n]) for k, o in enumerate(tail)]
            cols.append((parts[0] + last[0]) + (last[1] + last[2]))
        x = x + jnp.concatenate(cols, axis=1)

        y, y2 = _ln_twice(x)
        y2 = _round_bf16(y2)

        @pl.when(first)
        def _():
            wait_weight(w316, 1)

        h = jnp.concatenate([_mm(y2, w3[n]) for n in range(F // L)], axis=1)
        h = _round_bf16(jax.nn.gelu(h, approximate=True))

        @pl.when(first)
        def _():
            wait_weight(w416, 2)

        out = jnp.concatenate([_mm(h, w4[n]) for n in range(D // L)], axis=1)
        return x + (y + out)

    x_copy.wait()
    x0 = jnp.broadcast_to(xb[...].astype(jnp.float32), (8, D))
    x = lax.fori_loop(0, 2, layer, x0)
    o_ref[...] = x[:1].astype(o_ref.dtype)


@jax.jit
def pallas_interleave_layers__sliding_block_cached__mixer_s_mlp__decode_kernel(
    A_x: jax.Array,
    A_k_cache: jax.Array,
    A_v_cache: jax.Array,
    A_wq: jax.Array,
    A_wo: jax.Array,
    B_x: jax.Array,
    B_w1: jax.Array,
    B_w2: jax.Array,
    B_w3: jax.Array,
    B_w4: jax.Array,
):
    del B_x, B_w1, B_w2
    assert A_x.shape == (1, 1, D) and A_k_cache.shape == (1, NH, SK, DH)
    kt = jnp.swapaxes(A_k_cache, 2, 3).reshape(NH * DH, SK)
    vt = jnp.swapaxes(A_v_cache, 2, 3).reshape(NH * DH, SK)
    hbm = pl.BlockSpec(memory_space=pl.ANY)
    u32, f32 = jnp.uint32, jnp.float32
    out = pl.pallas_call(
        _kernel,
        out_shape=jax.ShapeDtypeStruct((1, D), A_x.dtype),
        in_specs=[hbm] * 7,
        scratch_shapes=[
            pltpu.VMEM((NP, NT, DH, L), u32),
            pltpu.VMEM((NP, NT, DH, L), u32),
            pltpu.VMEM((NH * DH // L, D // 2, L), u32),
            pltpu.VMEM((NP, D // L, DH, L), u32),
            pltpu.VMEM((F // L, D // 2, L), u32),
            pltpu.VMEM((D // L, F // 2, L), u32),
            pltpu.VMEM((1, D), A_x.dtype),
            pltpu.VMEM((NH * DH // L, 8, L), f32),
            pltpu.VMEM((NP * 15, 8, L), f32),
            *[pltpu.VMEM((8, 8, L), f32)] * 8,
            *[pltpu.VMEM((8, L), f32)] * 8,
            *[pltpu.VMEM((8, 8, L), f32)] * 2,
            *[pltpu.VMEM((2 * DH, L), f32)] * 2,
            *[pltpu.VMEM((3, 8, L), f32)] * 2,
            *[pltpu.VMEM((15, 8, L), f32)] * 2,
            *[pltpu.VMEM((3, L, L), f32)] * 2,
            *[pltpu.VMEM((8, 8, L), f32)] * U,
            pltpu.SemaphoreType.DMA((NP,)),
            pltpu.SemaphoreType.DMA((NP,)),
            pltpu.SemaphoreType.DMA((NP,)),
            pltpu.SemaphoreType.DMA((4,)),
        ],
        compiler_params=pltpu.CompilerParams(
            vmem_limit_bytes=120 * 2**20,
            disable_bounds_checks=True,
            disable_semaphore_checks=True,
            flags=None,
        ),
        name="interleave_decode",
    )(A_x.reshape(1, D), kt, vt, A_wq, A_wo, B_w3, B_w4)
    return out.reshape(1, 1, D)
```

```python
import jax
X = 'xfpaqo12bg'; XL = 'xfpon12g'
import jax.numpy as jnp
from jax import lax
import jax.experimental.pallas as pl
import jax.experimental.pallas.tpu as pltpu

D = 640
NH = 32
DH = 192
SK = 32768
W = 4096
F = 1536
L = 128
NP = NH // 2
NT = W // L
S0 = SK - W
EPS = 1e-5
SCALE = DH ** -0.5
NN = (((1,), (0,)), ((), ()))
W4R = int('128')
W4C = F // W4R
CR = int('192')
WR = int('128')
WP = int('0')
NTD = (((1,), (1,)), ((), ()))
U = 4


def _ln(x):
    m = jnp.sum(x, axis=-1, keepdims=True) * (1.0 / D)
    d = x - m
    v = jnp.sum(d * d, axis=-1, keepdims=True) * (1.0 / D)
    return d * lax.rsqrt(v + EPS)


def _ln_twice(x):
    d = x - jnp.sum(x, axis=-1, keepdims=True) * (1.0 / D)
    m2 = jnp.sum(d, axis=-1, keepdims=True) * (1.0 / D)
    v = jnp.sum(d * d, axis=-1, keepdims=True) * (1.0 / D)
    r = lax.rsqrt(v + EPS)
    y = d * r
    v2 = (v - m2 * m2) * (r * r)
    return y, (y - m2 * r) * lax.rsqrt(v2 + EPS)


def _round_bf16(x):
    return x.astype(jnp.bfloat16).astype(jnp.float32)


def _mm(lhs, w32):
    return lax.dot_general(lhs, pltpu.bitcast(w32, jnp.bfloat16), NN,
                           preferred_element_type=jnp.float32)


def _when(cond):
    if isinstance(cond, bool):
        return (lambda f: f()) if cond else (lambda f: None)
    return pl.when(cond)


def _kernel(x_hbm, k_hbm, v_hbm, wq_hbm, wo_hbm, w3_hbm, w4_hbm, o_ref,
            kb, vb, wq, wo, w3, w4, xb, qs, opart, *rest):
    sa, sb, lb, mb, rest = rest[0:4], rest[4:8], rest[8:12], rest[12:16], rest[16:]
    pb, acc, ob, qpart, tb, rest = (*(rest[2 * t:2 * t + 2] for t in range(5)), rest[10:])
    nb, (ksem, vsem, osem, w4sem, wsem) = rest[:U], rest[U:]
    kb16, vb16 = kb.bitcast(jnp.bfloat16), vb.bitcast(jnp.bfloat16)
    wq16, wo16 = wq.bitcast(jnp.bfloat16), wo.bitcast(jnp.bfloat16)
    w316, w416 = w3.bitcast(jnp.bfloat16), w4.bitcast(jnp.bfloat16)
    PR = 2 * DH

    def pair_row(ip):
        return ip * PR if isinstance(ip, int) else pl.multiple_of(ip * PR, L)

    def start_cache(hbm, dst16, sem, ip):
        r0 = pair_row(ip)
        for j in range(NT):
            for b in range(PR // CR):
                pltpu.make_async_copy(hbm.at[pl.ds(r0 + b * CR, CR), pl.ds(S0 + j * L, L)],
                                      dst16.at[ip, j, pl.ds(b * CR, CR)],
                                      sem.at[ip]).start(priority=b % 2)

    def start_wo(ip):
        r0 = pair_row(ip)
        for n in range(D // L):
            for b in range(2):
                pltpu.make_async_copy(wo_hbm.at[pl.ds(r0 + b * DH, DH), pl.ds(n * L, L)],
                                      wo16.at[ip, n, pl.ds(b * DH, DH)],
                                      osem.at[ip]).start(priority=b if WP else 0)

    def wait_slab(dst16, sem, ip):
        pltpu.make_async_copy(dst16.at[ip], dst16.at[ip], sem.at[ip]).wait()

    def start_weight(hbm, dst16, s, rows):
        for r in range(0, dst16.shape[1], rows):
            for n in range(dst16.shape[0]):
                pltpu.make_async_copy(hbm.at[pl.ds(r, rows), pl.ds(n * L, L)],
                                      dst16.at[n, pl.ds(r, rows)],
                                      wsem.at[s]).start(priority=n % 2 if WP else 0)

    def start_w4():
        for c in range(W4C):
            for n in range(D // L):
                pltpu.make_async_copy(w4_hbm.at[pl.ds(c * W4R, W4R), pl.ds(n * L, L)],
                                      w416.at[c, n], w4sem.at[c]).start(priority=(c + n) % 2 if WP else 0)

    def wait_weight(dst16, s):
        pltpu.make_async_copy(dst16, dst16, wsem.at[s]).wait()

    x_copy = pltpu.make_async_copy(x_hbm, xb, wsem.at[2])
    x_copy.start()
    start_weight(wq_hbm, wq16, 0, WR)
    for i in range(4):
        start_cache(k_hbm, kb16, ksem, i)
    start_cache(v_hbm, vb16, vsem, 0)
    start_cache(k_hbm, kb16, ksem, 4)

    row = lax.broadcasted_iota(jnp.int32, (8, L), 0)
    lane = lax.broadcasted_iota(jnp.int32, (8, L), 1)
    mid_mask = (row % 2 == 0) == (lane < L // 2)

    def put_q(ip, n, q):
        q = _round_bf16(q)
        qs[ip * 3 + n] = jnp.where(mid_mask, q, 0.0) if n == 1 else q

    def q_partials(z, ip, buf):
        for n in range(3):
            for kt in range(D // L):
                buf[n * 5 + kt] = _mm(z[:, kt * L:(kt + 1) * L],
                                      wq[ip * 3 + n, kt * 64:(kt + 1) * 64, :])

    def q_sum(ip, buf):
        for n in range(3):
            t = [buf[n * 5 + kt] for kt in range(D // L)]
            put_q(ip, n, (t[0] + t[1]) + (t[2] + t[3]) + t[4])

    def qk(ip, a_ref, b_ref):
        lhs = [qs[ip * 3 + kt] for kt in range(3)]
        for j in range(NT):
            J, v = divmod(j, 4)
            r = [_mm(lhs[kt], kb[ip, j, kt * 64:(kt + 1) * 64, :]) for kt in range(3)]
            a_ref[J, 2 * v:2 * v + 1, :] = r[0][2 * v:2 * v + 1, :]
            b_ref[J, 2 * v:2 * v + 2, :] = r[1][2 * v:2 * v + 2, :]
            a_ref[J, 2 * v + 1:2 * v + 2, :] = r[2][2 * v + 1:2 * v + 2, :]

    def per_head(t, op):
        t = op(t, pltpu.roll(t, 2, 0))
        return op(t, pltpu.roll(t, 4, 0))

    def score_max(a_ref, b_ref, m_ref):
        s = [(a_ref[J] + b_ref[J]) * SCALE for J in range(8)]
        m = s[0]
        for t in s[1:]:
            m = jnp.maximum(m, t)
        for J in range(8):
            a_ref[J] = s[J]
        m_ref[...] = m

    def lane_max(m_ref):
        m_ref[...] = jnp.broadcast_to(jnp.max(m_ref[...], axis=1, keepdims=True), (8, L))

    def lane_sum(l_ref):
        l_ref[...] = jnp.broadcast_to(jnp.sum(l_ref[...], axis=1, keepdims=True), (8, L))

    def score_exp(a_ref, m_ref, p_ref, l_ref):
        m = per_head(m_ref[...], jnp.maximum)
        e = [jnp.exp(a_ref[J] - m) for J in range(8)]
        tot = e[0]
        for t in e[1:]:
            tot = tot + t
        for J in range(8):
            p_ref[J] = e[J]
        l_ref[...] = tot

    def pv(ip, p_ref, acc_ref, rows=PR):
        for h in range(2):
            nt = min(DH, rows - h * DH) // 16
            a = None
            for j in range(NT):
                r = 2 * (j % 4) + h
                p = jnp.broadcast_to(p_ref[j // 4, r:r + 1, :], (16, L))
                new = []
                for t in range(nt):
                    w = vb[ip, j, h * 96 + t * 8:h * 96 + t * 8 + 8, :]
                    f = pltpu.bitcast(w, jnp.bfloat16).astype(jnp.float32) * p
                    new.append(f if a is None else a[t] + f)
                a = new
            for t in range(nt):
                acc_ref[h * DH + t * 16:h * DH + t * 16 + 16, :] = a[t]

    def pv_mxu(ip, p_ref, n_ref):
        for J in range(8):
            lhs = _round_bf16(p_ref[J])
            for v in range(4):
                w = pltpu.bitcast(vb[ip, 4 * J + v, 128:192, :], jnp.bfloat16)
                r = lax.dot_general(lhs, w, NTD, preferred_element_type=jnp.float32)
                n_ref[J, 2 * v + 1:2 * v + 2, :] = r[2 * v + 1:2 * v + 2, :]

    def transpose_acc(acc_ref, t_ref, tiles=3):
        for kt in range(tiles):
            t_ref[kt] = acc_ref[kt * L:(kt + 1) * L, :].T

    def finalize(t_ref, l_ref, n_ref=None):
        o = [jnp.sum(t_ref[kt], axis=0, keepdims=True) for kt in range(3 if n_ref is None else 2)]
        if n_ref is not None:
            t = [jnp.where(row % 2 == 1, n_ref[J], 0.0) for J in range(8)]
            t = ((t[0] + t[1]) + (t[2] + t[3])) + ((t[4] + t[5]) + (t[6] + t[7]))
            o.append(jnp.sum(t, axis=0, keepdims=True))
        o = jnp.concatenate(o, axis=1)
        o = jnp.broadcast_to(o, (8, PR))
        inv = 1.0 / per_head(l_ref[...], jnp.add)
        i0, i1 = jnp.broadcast_to(inv[0:1], (8, L)), jnp.broadcast_to(inv[1:2], (8, L))
        sc = (i0, jnp.where(lane < L // 2, i0, i1), i1)
        return [_round_bf16(o[:, kt * L:(kt + 1) * L] * sc[kt]) for kt in range(3)]

    def o_partials(ip, o_tiles):
        for kt in range(3):
            lhs = o_tiles[kt]
            for n in range(D // L):
                opart[ip * 15 + kt * 5 + n] = _mm(lhs, wo[ip, n, kt * 64:(kt + 1) * 64, :])

    def layer(li, x):
        first = li == 0
        z = _round_bf16(_ln(x))

        @pl.when(first)
        def _():
            wait_weight(wq16, 0)
            for i in range(4):
                wait_slab(kb16, ksem, i)
            start_cache(v_hbm, vb16, vsem, 1)

        for i in range(5):
            for n in range(3):
                put_q(i, n, _mm(z, wq[i * 3 + n]))
        q_partials(z, 5, qpart[0])
        for i in range(4):
            qk(i, sa[i], sb[i])
        for i in range(3):
            score_max(sa[i], sb[i], mb[i])
        for i in range(2):
            lane_max(mb[i])
        score_exp(sa[0], mb[0], pb[0], lb[0])
        acc[1][...] = jnp.zeros(acc[1].shape, jnp.float32)
        tb[0][...] = jnp.zeros(tb[0].shape, jnp.float32)
        lb[2][...] = jnp.ones(lb[2].shape, jnp.float32)
        lb[3][...] = jnp.ones(lb[3].shape, jnp.float32)
        ob[1][...] = jnp.zeros(ob[1].shape, jnp.float32)

        def stage(i, u, last):
            if True:

                @pl.when(first)
                def _():
                    wait_slab(vb16, vsem, i)

                    @_when(i + 5 < NP)
                    def _():
                        start_cache(k_hbm, kb16, ksem, i + 5)

                    start_wo(i)

                    @_when(i >= 3)
                    def _():
                        wait_slab(wo16, osem, i - 3)

                    if last and u == (NP - 2) % U:
                        @_when(i == NP - 2)
                        def _():
                            start_weight(w3_hbm, w316, 1, WR)

                    if last and u == (NP - 1) % U:
                        @_when(i == NP - 1)
                        def _():
                            start_w4()

                    @_when(i + 4 < NP)
                    def _():
                        wait_slab(kb16, ksem, i + 4)

                    @_when(i + 2 < NP)
                    def _():
                        start_cache(v_hbm, vb16, vsem, i + 2)

                for c_ in (XL if last else X):
                    if c_ == "f":
                        transpose_acc(acc[(u + 1) % 2], tb[(u + 1) % 2], 2 if last and u >= 1 else 3)
                    if c_ == "g":
                        o = finalize(tb[u % 2], lb[(u + 2) % 4], nb[u - 2] if last and u >= 2 else None)
                        for kt in range(3):
                            ob[u % 2][kt] = o[kt]
                    if c_ == "p":
                        pv(i, pb[u % 2], acc[u % 2], 2 * L if last else PR)
                    if c_ == "n":
                        pv_mxu(i, pb[u % 2], nb[u])
                    if c_ == "q":
                        qk(jnp.minimum(i + 4, NP - 1), sa[u % 4], sb[u % 4])
                    if c_ == "1" and (not last or u < 1):
                        score_max(sa[(u + 3) % 4], sb[(u + 3) % 4], mb[(u + 3) % 4])
                    if c_ == "x":
                        if not last or u < 2:
                            lane_max(mb[(u + 2) % 4])
                        lane_sum(lb[u % 4])
                    if c_ == "2" and (not last or u < 3):
                        score_exp(sa[(u + 1) % 4], mb[(u + 1) % 4], pb[(u + 1) % 2], lb[(u + 1) % 4])
                    if c_ == "a":
                        q_partials(z, jnp.minimum(i + 6, NP - 1), qpart[(u + 1) % 2])
                    if c_ == "b":
                        q_sum(jnp.minimum(i + 5, NP - 1), qpart[u % 2])
                    if c_ == "o":
                        o_partials((i - 3 if last else jnp.maximum(i - 3, 0)), [ob[(u + 1) % 2][kt] for kt in range(3)])

        def stages(t, c):
            for u in range(U):
                stage(t * U + u, u, False)
            return c

        lax.fori_loop(0, NP // U - 1, stages, 0)
        for u in range(U):
            stage(NP - U + u, u, True)

        @pl.when(first)
        def _():
            for ip in range(NP - 3, NP):
                wait_slab(wo16, osem, ip)

        transpose_acc(acc[1], tb[1], 2)
        tail = ([ob[1][kt] for kt in range(3)],
                finalize(tb[0], lb[2], nb[2]), finalize(tb[1], lb[3], nb[3]))
        cols = []
        for n in range(D // L):
            parts = [opart[t * 5 + n] for t in range(3 * (NP - 3))]
            while len(parts) > 1:
                parts = [sum(parts[k:k + 2][1:], parts[k]) for k in range(0, len(parts), 2)]
            last = [_mm(jnp.concatenate(o, axis=1), wo[NP - 3 + k, n]) for k, o in enumerate(tail)]
            cols.append((parts[0] + last[0]) + (last[1] + last[2]))
        x = x + jnp.concatenate(cols, axis=1)

        y, y2 = _ln_twice(x)
        y2 = _round_bf16(y2)

        def mlp(wait):
            if wait:
                wait_weight(w316, 1)
            h = [_round_bf16(jax.nn.gelu(_mm(y2, w3[n]), approximate=True)) for n in range(F // L)]
            cols = [None] * (D // L)
            for c in range(W4C):
                if wait:
                    wait_slab(w416, w4sem, c)
                for kk in range(W4R // L):
                    for n in range(D // L):
                        r = _mm(h[c * W4R // L + kk], w4[c, n, kk * 64:(kk + 1) * 64, :])
                        cols[n] = r if cols[n] is None else cols[n] + r
            return jnp.concatenate(cols, axis=1)

        out = lax.cond(first, lambda: mlp(True), lambda: mlp(False))
        return x + (y + out)

    x_copy.wait()
    x0 = jnp.broadcast_to(xb[...].astype(jnp.float32), (8, D))
    x = lax.fori_loop(0, 2, layer, x0)
    o_ref[...] = x[:1].astype(o_ref.dtype)


@jax.jit
def pallas_interleave_layers__sliding_block_cached__mixer_s_mlp__decode_kernel(
    A_x: jax.Array,
    A_k_cache: jax.Array,
    A_v_cache: jax.Array,
    A_wq: jax.Array,
    A_wo: jax.Array,
    B_x: jax.Array,
    B_w1: jax.Array,
    B_w2: jax.Array,
    B_w3: jax.Array,
    B_w4: jax.Array,
):
    del B_x, B_w1, B_w2
    assert A_x.shape == (1, 1, D) and A_k_cache.shape == (1, NH, SK, DH)
    kt = jnp.swapaxes(A_k_cache, 2, 3).reshape(NH * DH, SK)
    vt = jnp.swapaxes(A_v_cache, 2, 3).reshape(NH * DH, SK)
    hbm = pl.BlockSpec(memory_space=pl.ANY)
    u32, f32 = jnp.uint32, jnp.float32
    out = pl.pallas_call(
        _kernel,
        out_shape=jax.ShapeDtypeStruct((1, D), A_x.dtype),
        in_specs=[hbm] * 7,
        scratch_shapes=[
            pltpu.VMEM((NP, NT, DH, L), u32),
            pltpu.VMEM((NP, NT, DH, L), u32),
            pltpu.VMEM((NH * DH // L, D // 2, L), u32),
            pltpu.VMEM((NP, D // L, DH, L), u32),
            pltpu.VMEM((F // L, D // 2, L), u32),
            pltpu.VMEM((W4C, D // L, W4R // 2, L), u32),
            pltpu.VMEM((1, D), A_x.dtype),
            pltpu.VMEM((NH * DH // L, 8, L), f32),
            pltpu.VMEM((NP * 15, 8, L), f32),
            *[pltpu.VMEM((8, 8, L), f32)] * 8,
            *[pltpu.VMEM((8, L), f32)] * 8,
            *[pltpu.VMEM((8, 8, L), f32)] * 2,
            *[pltpu.VMEM((2 * DH, L), f32)] * 2,
            *[pltpu.VMEM((3, 8, L), f32)] * 2,
            *[pltpu.VMEM((15, 8, L), f32)] * 2,
            *[pltpu.VMEM((3, L, L), f32)] * 2,
            *[pltpu.VMEM((8, 8, L), f32)] * U,
            pltpu.SemaphoreType.DMA((NP,)),
            pltpu.SemaphoreType.DMA((NP,)),
            pltpu.SemaphoreType.DMA((NP,)),
            pltpu.SemaphoreType.DMA((W4C,)),
            pltpu.SemaphoreType.DMA((3,)),
        ],
        compiler_params=pltpu.CompilerParams(
            vmem_limit_bytes=120 * 2**20,
            disable_bounds_checks=True,
            disable_semaphore_checks=True,
            flags=None,
        ),
        name="interleave_decode",
    )(A_x.reshape(1, D), kt, vt, A_wq, A_wo, B_w3, B_w4)
    return out.reshape(1, 1, D)
```

```python
import jax
import jax.numpy as jnp
from jax import lax
import jax.experimental.pallas as pl
import jax.experimental.pallas.tpu as pltpu

D = 640
NH = 32
DH = 192
SK = 32768
W = 4096
F = 1536
L = 128
NP = NH // 2
PR = 2 * DH
NT = W // L
U = 4
S0 = SK - W
EPS = 1e-5
SCALE = DH ** -0.5
W4_ORDER = [c + b * (F // L // 2) for c in range(F // L // 2) for b in range(2)]
KSEM, VSEM, W4SEM = 0, NP, 2 * NP
WQSEM, WOSEM, W3SEM, XSEM = (W4SEM + F // L + s for s in range(4))


def _ln(x):
    m = jnp.sum(x, axis=-1, keepdims=True) * (1.0 / D)
    d = x - m
    v = jnp.sum(d * d, axis=-1, keepdims=True) * (1.0 / D)
    return d * lax.rsqrt(v + EPS)


def _ln_twice(x):
    d = x - jnp.sum(x, axis=-1, keepdims=True) * (1.0 / D)
    m2 = jnp.sum(d, axis=-1, keepdims=True) * (1.0 / D)
    v = jnp.sum(d * d, axis=-1, keepdims=True) * (1.0 / D)
    r = lax.rsqrt(v + EPS)
    y = d * r
    v2 = (v - m2 * m2) * (r * r)
    return y, (y - m2 * r) * lax.rsqrt(v2 + EPS)


def _round_bf16(x):
    return x.astype(jnp.bfloat16).astype(jnp.float32)


def _mm(lhs, w32, contract=0):
    return lax.dot_general(lhs, pltpu.bitcast(w32, jnp.bfloat16),
                           (((1,), (contract,)), ((), ())), preferred_element_type=jnp.float32)


def _tree_sum(xs):
    while len(xs) > 1:
        xs = [xs[k] + xs[k + 1] if k + 1 < len(xs) else xs[k] for k in range(0, len(xs), 2)]
    return xs[0]


def _when(cond):
    if isinstance(cond, bool):
        return (lambda f: f()) if cond else (lambda f: None)
    return pl.when(cond)


def _kernel(x_hbm, k_hbm, v_hbm, wq_hbm, wo_hbm, w3_hbm, w4_hbm, o_ref,
            kb, vb, wq, wo, w3, w4, xb, qs, opart, *rest):
    sa, sb, lb, mb, nb = (rest[4 * t:4 * t + 4] for t in range(5))
    pb, acc, tb, ob, qpart = (rest[20 + 2 * t:22 + 2 * t] for t in range(5))
    sems = rest[30]
    kb16, vb16 = kb.bitcast(jnp.bfloat16), vb.bitcast(jnp.bfloat16)
    wq16, wo16 = wq.bitcast(jnp.bfloat16), wo.bitcast(jnp.bfloat16)
    w316, w416 = w3.bitcast(jnp.bfloat16), w4.bitcast(jnp.bfloat16)

    def start_cache(hbm, dst16, sem, ip):
        r0 = ip * PR if isinstance(ip, int) else pl.multiple_of(ip * PR, L)
        for j in range(NT):
            for h in range(2):
                pltpu.make_async_copy(hbm.at[pl.ds(r0 + h * DH, DH), pl.ds(S0 + j * L, L)],
                                      dst16.at[ip, j, pl.ds(h * DH, DH)],
                                      sems.at[sem + ip]).start(priority=h)

    def start_wide(hbm, dst16, sem):
        for r in range(0, D, L):
            for n in range(dst16.shape[0]):
                pltpu.make_async_copy(hbm.at[pl.ds(r, L), pl.ds(n * L, L)],
                                      dst16.at[n, pl.ds(r, L)], sems.at[sem]).start(priority=n % 2)

    def start_wo():
        for ip in range(NP):
            for n in range(D // L):
                for h in range(2):
                    pltpu.make_async_copy(wo_hbm.at[pl.ds(ip * PR + h * DH, DH), pl.ds(n * L, L)],
                                          wo16.at[ip, n, pl.ds(h * DH, DH)],
                                          sems.at[WOSEM]).start(priority=h)

    def start_w4():
        for c in range(0, F // L, 2):
            for n in range(D // L):
                for b in range(2):
                    kt = W4_ORDER[c + b]
                    pltpu.make_async_copy(w4_hbm.at[pl.ds(kt * L, L), pl.ds(n * L, L)],
                                          w416.at[kt, n], sems.at[W4SEM + kt]).start(priority=b)

    def wait_all(dst16, sem):
        pltpu.make_async_copy(dst16, dst16, sems.at[sem]).wait()

    x_copy = pltpu.make_async_copy(x_hbm, xb, sems.at[XSEM])
    x_copy.start()
    start_wide(wq_hbm, wq16, WQSEM)
    start_wo()
    for i in range(4):
        start_cache(k_hbm, kb16, KSEM, i)
    start_cache(v_hbm, vb16, VSEM, 0)
    start_cache(k_hbm, kb16, KSEM, 4)

    row = lax.broadcasted_iota(jnp.int32, (8, L), 0)
    lane = lax.broadcasted_iota(jnp.int32, (8, L), 1)
    mid_mask = (row % 2 == 0) == (lane < L // 2)

    def put_q(ip, n, q):
        q = _round_bf16(q)
        qs[ip * 3 + n] = jnp.where(mid_mask, q, 0.0) if n == 1 else q

    def q_partials(z, ip, buf):
        for n in range(3):
            for kt in range(D // L):
                buf[n * 5 + kt] = _mm(z[:, kt * L:(kt + 1) * L],
                                      wq[ip * 3 + n, kt * 64:(kt + 1) * 64, :])

    def q_sum(ip, buf):
        for n in range(3):
            put_q(ip, n, _tree_sum([buf[n * 5 + kt] for kt in range(D // L)]))

    def qk(ip, a_ref, b_ref):
        lhs = [qs[ip * 3 + kt] for kt in range(3)]
        for j in range(NT):
            J, v = divmod(j, 4)
            r = [_mm(lhs[kt], kb[ip, j, kt * 64:(kt + 1) * 64, :]) for kt in range(3)]
            a_ref[J, 2 * v:2 * v + 1, :] = r[0][2 * v:2 * v + 1, :]
            b_ref[J, 2 * v:2 * v + 2, :] = r[1][2 * v:2 * v + 2, :]
            a_ref[J, 2 * v + 1:2 * v + 2, :] = r[2][2 * v + 1:2 * v + 2, :]

    def per_head(t, op):
        t = op(t, pltpu.roll(t, 2, 0))
        return op(t, pltpu.roll(t, 4, 0))

    def score_max(a_ref, b_ref, m_ref):
        s = [(a_ref[J] + b_ref[J]) * SCALE for J in range(8)]
        m = s[0]
        for t in s[1:]:
            m = jnp.maximum(m, t)
        for J in range(8):
            a_ref[J] = s[J]
        m_ref[...] = m

    def lane_max(m_ref):
        m_ref[...] = jnp.broadcast_to(jnp.max(m_ref[...], axis=1, keepdims=True), (8, L))

    def score_exp(a_ref, m_ref, p_ref, l_ref):
        m = per_head(m_ref[...], jnp.maximum)
        e = [jnp.exp(a_ref[J] - m) for J in range(8)]
        tot = e[0]
        for t in e[1:]:
            tot = tot + t
        for J in range(8):
            p_ref[J] = e[J]
        l_ref[...] = tot

    def lane_sum(l_ref):
        l_ref[...] = jnp.broadcast_to(jnp.sum(l_ref[...], axis=1, keepdims=True), (8, L))

    def pv(ip, p_ref, acc_ref, rows):
        for h in range(2):
            nt = min(DH, rows - h * DH) // 16
            a = None
            for j in range(NT):
                r = 2 * (j % 4) + h
                p = jnp.broadcast_to(p_ref[j // 4, r:r + 1, :], (16, L))
                new = []
                for t in range(nt):
                    w = vb[ip, j, h * 96 + t * 8:h * 96 + t * 8 + 8, :]
                    f = pltpu.bitcast(w, jnp.bfloat16).astype(jnp.float32) * p
                    new.append(f if a is None else a[t] + f)
                a = new
            for t in range(nt):
                acc_ref[h * DH + t * 16:h * DH + t * 16 + 16, :] = a[t]

    def pv_mxu(ip, p_ref, n_ref):
        for J in range(8):
            lhs = _round_bf16(p_ref[J])
            for v in range(4):
                r = _mm(lhs, vb[ip, 4 * J + v, 2 * 64:3 * 64, :], contract=1)
                n_ref[J, 2 * v + 1:2 * v + 2, :] = r[2 * v + 1:2 * v + 2, :]

    def transpose_acc(acc_ref, t_ref, tiles):
        for kt in range(tiles):
            t_ref[kt] = acc_ref[kt * L:(kt + 1) * L, :].T

    def finalize(t_ref, l_ref, n_ref=None):
        o = [jnp.sum(t_ref[kt], axis=0, keepdims=True) for kt in range(3 if n_ref is None else 2)]
        if n_ref is not None:
            t = _tree_sum([jnp.where(row % 2 == 1, n_ref[J], 0.0) for J in range(8)])
            o.append(jnp.sum(t, axis=0, keepdims=True))
        inv = 1.0 / per_head(l_ref[...], jnp.add)
        i0, i1 = jnp.broadcast_to(inv[0:1], (8, L)), jnp.broadcast_to(inv[1:2], (8, L))
        sc = (i0, jnp.where(lane < L // 2, i0, i1), i1)
        return [_round_bf16(jnp.broadcast_to(o[kt], (8, L)) * sc[kt]) for kt in range(3)]

    def o_partials(ip, o_tiles):
        for kt in range(3):
            for n in range(D // L):
                opart[ip * 15 + kt * 5 + n] = _mm(o_tiles[kt], wo[ip, n, kt * 64:(kt + 1) * 64, :])

    def layer(li, x):
        first = li == 0
        z = _round_bf16(_ln(x))

        @pl.when(first)
        def _():
            wait_all(wq16, WQSEM)
            wait_all(wo16, WOSEM)
            for i in range(4):
                wait_all(kb16.at[i], KSEM + i)
            start_cache(v_hbm, vb16, VSEM, 1)

        for i in range(5):
            for n in range(3):
                put_q(i, n, _mm(z, wq[i * 3 + n]))
        q_partials(z, 5, qpart[0])
        for i in range(4):
            qk(i, sa[i], sb[i])
        for i in range(3):
            score_max(sa[i], sb[i], mb[i])
        for i in range(2):
            lane_max(mb[i])
        score_exp(sa[0], mb[0], pb[0], lb[0])
        acc[1][...] = jnp.zeros(acc[1].shape, jnp.float32)
        tb[0][...] = jnp.zeros(tb[0].shape, jnp.float32)
        lb[2][...] = jnp.ones(lb[2].shape, jnp.float32)
        lb[3][...] = jnp.ones(lb[3].shape, jnp.float32)
        ob[1][...] = jnp.zeros(ob[1].shape, jnp.float32)

        def stage(i, u, last):
            @pl.when(first)
            def _():
                wait_all(vb16.at[i], VSEM + i)

                @_when(i + 5 < NP)
                def _():
                    start_cache(k_hbm, kb16, KSEM, i + 5)

                if last and u == U - 2:
                    start_wide(w3_hbm, w316, W3SEM)

                @_when(i + 4 < NP)
                def _():
                    wait_all(kb16.at[i + 4], KSEM + i + 4)

                @_when(i + 2 < NP)
                def _():
                    start_cache(v_hbm, vb16, VSEM, i + 2)

            if not last or u < 2:
                lane_max(mb[(u + 2) % 4])
            lane_sum(lb[u % 4])
            transpose_acc(acc[(u + 1) % 2], tb[(u + 1) % 2], 2 if last and u >= 1 else 3)
            pv(i, pb[u % 2], acc[u % 2], 2 * L if last else PR)
            o_prev = [ob[(u + 1) % 2][kt] for kt in range(3)]
            if last:
                o_partials(i - 3, o_prev)
                pv_mxu(i, pb[u % 2], nb[u])
            else:
                q_partials(z, jnp.minimum(i + 6, NP - 1), qpart[(u + 1) % 2])
                qk(jnp.minimum(i + 4, NP - 1), sa[u % 4], sb[u % 4])
                o_partials(jnp.maximum(i - 3, 0), o_prev)
            if not last or u < 1:
                score_max(sa[(u + 3) % 4], sb[(u + 3) % 4], mb[(u + 3) % 4])
            if not last or u < 3:
                score_exp(sa[(u + 1) % 4], mb[(u + 1) % 4], pb[(u + 1) % 2], lb[(u + 1) % 4])
            if not last:
                q_sum(jnp.minimum(i + 5, NP - 1), qpart[u % 2])
            o = finalize(tb[u % 2], lb[(u + 2) % 4], nb[u - 2] if last and u >= 2 else None)
            for kt in range(3):
                ob[u % 2][kt] = o[kt]

        def stages(t, c):
            for u in range(U):
                stage(t * U + u, u, False)
            return c

        lax.fori_loop(0, NP // U - 1, stages, 0)
        for u in range(U):
            stage(NP - U + u, u, True)

        pl.when(first)(start_w4)

        transpose_acc(acc[1], tb[1], 2)
        tail = ([ob[1][kt] for kt in range(3)],
                finalize(tb[0], lb[2], nb[2]), finalize(tb[1], lb[3], nb[3]))
        cols = []
        for n in range(D // L):
            done = _tree_sum([opart[t * 5 + n] for t in range(3 * (NP - 3))])
            rest_ = [_mm(jnp.concatenate(o, axis=1), wo[NP - 3 + k, n]) for k, o in enumerate(tail)]
            cols.append((done + rest_[0]) + (rest_[1] + rest_[2]))
        x = x + jnp.concatenate(cols, axis=1)

        y, y2 = _ln_twice(x)
        y2 = _round_bf16(y2)

        def mlp(wait):
            if wait:
                wait_all(w316, W3SEM)
            h = [_round_bf16(jax.nn.gelu(_mm(y2, w3[n]), approximate=True)) for n in range(F // L)]
            cols = [None] * (D // L)
            for kt in W4_ORDER:
                if wait:
                    wait_all(w416.at[kt], W4SEM + kt)
                for n in range(D // L):
                    r = _mm(h[kt], w4[kt, n])
                    cols[n] = r if cols[n] is None else cols[n] + r
            return jnp.concatenate(cols, axis=1)

        return x + (y + lax.cond(first, lambda: mlp(True), lambda: mlp(False)))

    x_copy.wait()
    x0 = jnp.broadcast_to(xb[...].astype(jnp.float32), (8, D))
    x = lax.fori_loop(0, 2, layer, x0)
    o_ref[...] = x[:1].astype(o_ref.dtype)


@jax.jit
def pallas_interleave_layers__sliding_block_cached__mixer_s_mlp__decode_kernel(
    A_x: jax.Array,
    A_k_cache: jax.Array,
    A_v_cache: jax.Array,
    A_wq: jax.Array,
    A_wo: jax.Array,
    B_x: jax.Array,
    B_w1: jax.Array,
    B_w2: jax.Array,
    B_w3: jax.Array,
    B_w4: jax.Array,
):
    del B_x, B_w1, B_w2
    assert A_x.shape == (1, 1, D) and A_k_cache.shape == (1, NH, SK, DH)
    kt = jnp.swapaxes(A_k_cache, 2, 3).reshape(NH * DH, SK)
    vt = jnp.swapaxes(A_v_cache, 2, 3).reshape(NH * DH, SK)
    u32, f32 = jnp.uint32, jnp.float32
    out = pl.pallas_call(
        _kernel,
        out_shape=jax.ShapeDtypeStruct((1, D), A_x.dtype),
        in_specs=[pl.BlockSpec(memory_space=pl.ANY)] * 7,
        scratch_shapes=[
            pltpu.VMEM((NP, NT, DH, L), u32),
            pltpu.VMEM((NP, NT, DH, L), u32),
            pltpu.VMEM((NH * DH // L, D // 2, L), u32),
            pltpu.VMEM((NP, D // L, DH, L), u32),
            pltpu.VMEM((F // L, D // 2, L), u32),
            pltpu.VMEM((F // L, D // L, L // 2, L), u32),
            pltpu.VMEM((1, D), A_x.dtype),
            pltpu.VMEM((NH * DH // L, 8, L), f32),
            pltpu.VMEM((NP * 15, 8, L), f32),
            *[pltpu.VMEM((8, 8, L), f32)] * 8,
            *[pltpu.VMEM((8, L), f32)] * 8,
            *[pltpu.VMEM((8, 8, L), f32)] * 4,
            *[pltpu.VMEM((8, 8, L), f32)] * 2,
            *[pltpu.VMEM((PR, L), f32)] * 2,
            *[pltpu.VMEM((3, L, L), f32)] * 2,
            *[pltpu.VMEM((3, 8, L), f32)] * 2,
            *[pltpu.VMEM((15, 8, L), f32)] * 2,
            pltpu.SemaphoreType.DMA((XSEM + 1,)),
        ],
        compiler_params=pltpu.CompilerParams(
            vmem_limit_bytes=120 * 2**20,
            disable_bounds_checks=True,
            disable_semaphore_checks=True,
        ),
        name="interleave_decode",
    )(A_x.reshape(1, D), kt, vt, A_wq, A_wo, B_w3, B_w4)
    return out.reshape(1, 1, D)
```

```python
import jax
import jax.numpy as jnp
from jax import lax
import jax.experimental.pallas as pl
import jax.experimental.pallas.tpu as pltpu

D = 640
NH = 32
DH = 192
SK = 32768
W = 4096
F = 1536
L = 128
NP = NH // 2
PR = 2 * DH
NT = W // L
U = 4
S0 = SK - W
EPS = 1e-5
SCALE = DH ** -0.5
W4_ORDER = [c + b * (F // L // 2) for c in range(F // L // 2) for b in range(2)]
KSEM, VSEM, W4SEM = 0, NP, 2 * NP
WQSEM, WOSEM, W3SEM, XSEM = (W4SEM + F // L + s for s in range(4))


def _ln(x):
    m = jnp.sum(x, axis=-1, keepdims=True) * (1.0 / D)
    d = x - m
    v = jnp.sum(d * d, axis=-1, keepdims=True) * (1.0 / D)
    return d * lax.rsqrt(v + EPS)


def _ln_twice(x):
    d = x - jnp.sum(x, axis=-1, keepdims=True) * (1.0 / D)
    m2 = jnp.sum(d, axis=-1, keepdims=True) * (1.0 / D)
    v = jnp.sum(d * d, axis=-1, keepdims=True) * (1.0 / D)
    r = lax.rsqrt(v + EPS)
    y = d * r
    v2 = (v - m2 * m2) * (r * r)
    return y, (y - m2 * r) * lax.rsqrt(v2 + EPS)


def _round_bf16(x):
    return x.astype(jnp.bfloat16).astype(jnp.float32)


def _mm(lhs, w32, contract=0):
    return lax.dot_general(lhs, pltpu.bitcast(w32, jnp.bfloat16),
                           (((1,), (contract,)), ((), ())), preferred_element_type=jnp.float32)


def _tree_sum(xs):
    while len(xs) > 1:
        xs = [xs[k] + xs[k + 1] if k + 1 < len(xs) else xs[k] for k in range(0, len(xs), 2)]
    return xs[0]


def _when(cond):
    if isinstance(cond, bool):
        return (lambda f: f()) if cond else (lambda f: None)
    return pl.when(cond)


def _kernel(x_hbm, k_hbm, v_hbm, wq_hbm, wo_hbm, w3_hbm, w4_hbm, o_ref,
            kb, vb, wq, wo, w3, w4, xb, qs, opart, *rest):
    sa, sb, lb, mb, nb = (rest[4 * t:4 * t + 4] for t in range(5))
    pb, acc, tb, ob, qpart = (rest[20 + 2 * t:22 + 2 * t] for t in range(5))
    sems = rest[30]
    kb16, vb16 = kb.bitcast(jnp.bfloat16), vb.bitcast(jnp.bfloat16)
    wq16, wo16 = wq.bitcast(jnp.bfloat16), wo.bitcast(jnp.bfloat16)
    w316, w416 = w3.bitcast(jnp.bfloat16), w4.bitcast(jnp.bfloat16)

    def start_cache(hbm, dst16, sem, ip):
        r0 = ip * PR if isinstance(ip, int) else pl.multiple_of(ip * PR, L)
        for j in range(NT):
            for h in range(2):
                pltpu.make_async_copy(hbm.at[pl.ds(r0 + h * DH, DH), pl.ds(S0 + j * L, L)],
                                      dst16.at[ip, j, pl.ds(h * DH, DH)],
                                      sems.at[sem + ip]).start(priority=h)

    def start_wide(hbm, dst16, sem):
        for r in range(0, D, L):
            for n in range(dst16.shape[0]):
                pltpu.make_async_copy(hbm.at[pl.ds(r, L), pl.ds(n * L, L)],
                                      dst16.at[n, pl.ds(r, L)], sems.at[sem]).start(priority=n % 2)

    def start_wo():
        for ip in range(NP):
            for n in range(D // L):
                for h in range(2):
                    pltpu.make_async_copy(wo_hbm.at[pl.ds(ip * PR + h * DH, DH), pl.ds(n * L, L)],
                                          wo16.at[ip, n, pl.ds(h * DH, DH)],
                                          sems.at[WOSEM]).start(priority=h)

    def start_w4():
        for c in range(0, F // L, 2):
            for n in range(D // L):
                for b in range(2):
                    kt = W4_ORDER[c + b]
                    pltpu.make_async_copy(w4_hbm.at[pl.ds(kt * L, L), pl.ds(n * L, L)],
                                          w416.at[kt, n], sems.at[W4SEM + kt]).start(priority=b)

    def wait_all(dst16, sem):
        pltpu.make_async_copy(dst16, dst16, sems.at[sem]).wait()

    x_copy = pltpu.make_async_copy(x_hbm, xb, sems.at[XSEM])
    x_copy.start()
    start_wide(wq_hbm, wq16, WQSEM)
    start_wo()
    for i in range(4):
        start_cache(k_hbm, kb16, KSEM, i)
    start_cache(v_hbm, vb16, VSEM, 0)
    start_cache(k_hbm, kb16, KSEM, 4)

    row = lax.broadcasted_iota(jnp.int32, (8, L), 0)
    lane = lax.broadcasted_iota(jnp.int32, (8, L), 1)
    mid_mask = (row % 2 == 0) == (lane < L // 2)

    def put_q(ip, n, q):
        q = _round_bf16(q)
        qs[ip * 3 + n] = jnp.where(mid_mask, q, 0.0) if n == 1 else q

    def q_partials(z, ip, buf):
        for n in range(3):
            for kt in range(D // L):
                buf[n * 5 + kt] = _mm(z[:, kt * L:(kt + 1) * L],
                                      wq[ip * 3 + n, kt * 64:(kt + 1) * 64, :])

    def q_sum(ip, buf):
        for n in range(3):
            put_q(ip, n, _tree_sum([buf[n * 5 + kt] for kt in range(D // L)]))

    def qk(ip, a_ref, b_ref):
        lhs = [qs[ip * 3 + kt] for kt in range(3)]
        for j in range(NT):
            J, v = divmod(j, 4)
            r = [_mm(lhs[kt], kb[ip, j, kt * 64:(kt + 1) * 64, :]) for kt in range(3)]
            a_ref[J, 2 * v:2 * v + 1, :] = r[0][2 * v:2 * v + 1, :]
            b_ref[J, 2 * v:2 * v + 2, :] = r[1][2 * v:2 * v + 2, :]
            a_ref[J, 2 * v + 1:2 * v + 2, :] = r[2][2 * v + 1:2 * v + 2, :]

    def per_head(t, op):
        t = op(t, pltpu.roll(t, 2, 0))
        return op(t, pltpu.roll(t, 4, 0))

    def score_max(a_ref, b_ref, m_ref):
        s = [(a_ref[J] + b_ref[J]) * SCALE for J in range(8)]
        m = s[0]
        for t in s[1:]:
            m = jnp.maximum(m, t)
        for J in range(8):
            a_ref[J] = s[J]
        m_ref[...] = m

    def lane_max(m_ref):
        m_ref[...] = jnp.broadcast_to(jnp.max(m_ref[...], axis=1, keepdims=True), (8, L))

    def score_exp(a_ref, m_ref, p_ref, l_ref):
        m = per_head(m_ref[...], jnp.maximum)
        e = [jnp.exp(a_ref[J] - m) for J in range(8)]
        tot = e[0]
        for t in e[1:]:
            tot = tot + t
        for J in range(8):
            p_ref[J] = e[J]
        l_ref[...] = tot

    def lane_sum(l_ref):
        l_ref[...] = jnp.broadcast_to(jnp.sum(l_ref[...], axis=1, keepdims=True), (8, L))

    def pv(ip, p_ref, acc_ref, rows):
        for h in range(2):
            nt = min(DH, rows - h * DH) // 16
            a = None
            for j in range(NT):
                r = 2 * (j % 4) + h
                p = jnp.broadcast_to(p_ref[j // 4, r:r + 1, :], (16, L))
                new = []
                for t in range(nt):
                    w = vb[ip, j, h * 96 + t * 8:h * 96 + t * 8 + 8, :]
                    f = pltpu.bitcast(w, jnp.bfloat16).astype(jnp.float32) * p
                    new.append(f if a is None else a[t] + f)
                a = new
            for t in range(nt):
                acc_ref[h * DH + t * 16:h * DH + t * 16 + 16, :] = a[t]

    def pv_mxu(ip, p_ref, n_ref):
        for J in range(8):
            lhs = _round_bf16(p_ref[J])
            for v in range(4):
                r = _mm(lhs, vb[ip, 4 * J + v, 2 * 64:3 * 64, :], contract=1)
                n_ref[J, 2 * v + 1:2 * v + 2, :] = r[2 * v + 1:2 * v + 2, :]

    def transpose_acc(acc_ref, t_ref, tiles):
        for kt in range(tiles):
            t_ref[kt] = acc_ref[kt * L:(kt + 1) * L, :].T

    def finalize(t_ref, l_ref, n_ref=None):
        o = [jnp.sum(t_ref[kt], axis=0, keepdims=True) for kt in range(3 if n_ref is None else 2)]
        if n_ref is not None:
            t = _tree_sum([jnp.where(row % 2 == 1, n_ref[J], 0.0) for J in range(8)])
            o.append(jnp.sum(t, axis=0, keepdims=True))
        inv = 1.0 / per_head(l_ref[...], jnp.add)
        i0, i1 = jnp.broadcast_to(inv[0:1], (8, L)), jnp.broadcast_to(inv[1:2], (8, L))
        sc = (i0, jnp.where(lane < L // 2, i0, i1), i1)
        return [_round_bf16(jnp.broadcast_to(o[kt], (8, L)) * sc[kt]) for kt in range(3)]

    def o_partials(ip, o_tiles):
        for kt in range(3):
            for n in range(D // L):
                opart[ip * 15 + kt * 5 + n] = _mm(o_tiles[kt], wo[ip, n, kt * 64:(kt + 1) * 64, :])

    def layer(li, x):
        first = li == 0
        z = _round_bf16(_ln(x))

        @pl.when(first)
        def _():
            wait_all(wq16, WQSEM)
            wait_all(wo16, WOSEM)
            for i in range(4):
                wait_all(kb16.at[i], KSEM + i)
            start_cache(v_hbm, vb16, VSEM, 1)

        for i in range(5):
            for n in range(3):
                put_q(i, n, _mm(z, wq[i * 3 + n]))
        q_partials(z, 5, qpart[0])
        for i in range(4):
            qk(i, sa[i], sb[i])
        for i in range(3):
            score_max(sa[i], sb[i], mb[i])
        for i in range(2):
            lane_max(mb[i])
        score_exp(sa[0], mb[0], pb[0], lb[0])
        acc[1][...] = jnp.zeros(acc[1].shape, jnp.float32)
        tb[0][...] = jnp.zeros(tb[0].shape, jnp.float32)
        lb[2][...] = jnp.ones(lb[2].shape, jnp.float32)
        lb[3][...] = jnp.ones(lb[3].shape, jnp.float32)
        ob[1][...] = jnp.zeros(ob[1].shape, jnp.float32)

        def stage(i, u, last):
            @pl.when(first)
            def _():
                wait_all(vb16.at[i], VSEM + i)

                @_when(i + 5 < NP)
                def _():
                    start_cache(k_hbm, kb16, KSEM, i + 5)

                if last and u == U - 2:
                    start_wide(w3_hbm, w316, W3SEM)

                @_when(i + 4 < NP)
                def _():
                    wait_all(kb16.at[i + 4], KSEM + i + 4)

                @_when(i + 2 < NP)
                def _():
                    start_cache(v_hbm, vb16, VSEM, i + 2)

            if not last or u < 2:
                lane_max(mb[(u + 2) % 4])
            lane_sum(lb[u % 4])
            transpose_acc(acc[(u + 1) % 2], tb[(u + 1) % 2], 2 if last and u >= 1 else 3)
            pv(i, pb[u % 2], acc[u % 2], 2 * L if last else PR)
            o_prev = [ob[(u + 1) % 2][kt] for kt in range(3)]
            if last:
                o_partials(i - 3, o_prev)
                pv_mxu(i, pb[u % 2], nb[u])
            else:
                q_partials(z, jnp.minimum(i + 6, NP - 1), qpart[(u + 1) % 2])
                qk(jnp.minimum(i + 4, NP - 1), sa[u % 4], sb[u % 4])
                o_partials(jnp.maximum(i - 3, 0), o_prev)
            if not last or u < 1:
                score_max(sa[(u + 3) % 4], sb[(u + 3) % 4], mb[(u + 3) % 4])
            if not last or u < 3:
                score_exp(sa[(u + 1) % 4], mb[(u + 1) % 4], pb[(u + 1) % 2], lb[(u + 1) % 4])
            if not last:
                q_sum(jnp.minimum(i + 5, NP - 1), qpart[u % 2])
            o = finalize(tb[u % 2], lb[(u + 2) % 4], nb[u - 2] if last and u >= 2 else None)
            for kt in range(3):
                ob[u % 2][kt] = o[kt]

        def stages(t, c):
            for u in range(U):
                stage(t * U + u, u, False)
            return c

        lax.fori_loop(0, NP // U - 1, stages, 0)
        for u in range(U):
            stage(NP - U + u, u, True)

        pl.when(first)(start_w4)

        transpose_acc(acc[1], tb[1], 2)
        tail = ([ob[1][kt] for kt in range(3)],
                finalize(tb[0], lb[2], nb[2]), finalize(tb[1], lb[3], nb[3]))
        rest_ = [[_mm(jnp.concatenate(o, axis=1), wo[NP - 3 + k, n]) for n in range(D // L)]
                 for k, o in enumerate(tail)]
        cols = [(_tree_sum([opart[t * 5 + n] for t in range(3 * (NP - 3))]) + rest_[0][n])
                + (rest_[1][n] + rest_[2][n]) for n in range(D // L)]
        x = x + jnp.concatenate(cols, axis=1)

        y, y2 = _ln_twice(x)
        y2 = _round_bf16(y2)

        def mlp(wait):
            if wait:
                wait_all(w316, W3SEM)
            h = [_round_bf16(jax.nn.gelu(_mm(y2, w3[n]), approximate=True)) for n in range(F // L)]
            cols = [None] * (D // L)
            for kt in W4_ORDER:
                if wait:
                    wait_all(w416.at[kt], W4SEM + kt)
                for n in range(D // L):
                    r = _mm(h[kt], w4[kt, n])
                    cols[n] = r if cols[n] is None else cols[n] + r
            return jnp.concatenate(cols, axis=1)

        return x + (y + lax.cond(first, lambda: mlp(True), lambda: mlp(False)))

    x_copy.wait()
    x0 = jnp.broadcast_to(xb[...].astype(jnp.float32), (8, D))
    x = lax.fori_loop(0, 2, layer, x0)
    o_ref[...] = x[:1].astype(o_ref.dtype)


@jax.jit
def pallas_interleave_layers__sliding_block_cached__mixer_s_mlp__decode_kernel(
    A_x: jax.Array,
    A_k_cache: jax.Array,
    A_v_cache: jax.Array,
    A_wq: jax.Array,
    A_wo: jax.Array,
    B_x: jax.Array,
    B_w1: jax.Array,
    B_w2: jax.Array,
    B_w3: jax.Array,
    B_w4: jax.Array,
):
    del B_x, B_w1, B_w2
    assert A_x.shape == (1, 1, D) and A_k_cache.shape == (1, NH, SK, DH)
    kt = jnp.swapaxes(A_k_cache, 2, 3).reshape(NH * DH, SK)
    vt = jnp.swapaxes(A_v_cache, 2, 3).reshape(NH * DH, SK)
    u32, f32 = jnp.uint32, jnp.float32
    out = pl.pallas_call(
        _kernel,
        out_shape=jax.ShapeDtypeStruct((1, D), A_x.dtype),
        in_specs=[pl.BlockSpec(memory_space=pl.ANY)] * 7,
        scratch_shapes=[
            pltpu.VMEM((NP, NT, DH, L), u32),
            pltpu.VMEM((NP, NT, DH, L), u32),
            pltpu.VMEM((NH * DH // L, D // 2, L), u32),
            pltpu.VMEM((NP, D // L, DH, L), u32),
            pltpu.VMEM((F // L, D // 2, L), u32),
            pltpu.VMEM((F // L, D // L, L // 2, L), u32),
            pltpu.VMEM((1, D), A_x.dtype),
            pltpu.VMEM((NH * DH // L, 8, L), f32),
            pltpu.VMEM((NP * 15, 8, L), f32),
            *[pltpu.VMEM((8, 8, L), f32)] * 8,
            *[pltpu.VMEM((8, L), f32)] * 8,
            *[pltpu.VMEM((8, 8, L), f32)] * 4,
            *[pltpu.VMEM((8, 8, L), f32)] * 2,
            *[pltpu.VMEM((PR, L), f32)] * 2,
            *[pltpu.VMEM((3, L, L), f32)] * 2,
            *[pltpu.VMEM((3, 8, L), f32)] * 2,
            *[pltpu.VMEM((15, 8, L), f32)] * 2,
            pltpu.SemaphoreType.DMA((XSEM + 1,)),
        ],
        compiler_params=pltpu.CompilerParams(
            vmem_limit_bytes=120 * 2**20,
            disable_bounds_checks=True,
            disable_semaphore_checks=True,
        ),
        name="interleave_decode",
    )(A_x.reshape(1, D), kt, vt, A_wq, A_wo, B_w3, B_w4)
    return out.reshape(1, 1, D)
```
